```python
import os as _os
_os.environ.setdefault('JAX_PLATFORMS', 'cpu')
import jax
import jax.numpy as jnp

def _softmax(x, axis=-1):
    return jax.nn.softmax(x, axis=axis)

def _gelu(x):
    return jax.nn.gelu(x, approximate=True)

def _silu(x):
    return jax.nn.silu(x)

def _sigmoid(x):
    return jax.nn.sigmoid(x)

def _layernorm(x, axis=-1, eps=1e-05):
    m = jnp.mean(x, axis=axis, keepdims=True)
    v = jnp.var(x, axis=axis, keepdims=True)
    return (x - m) / jnp.sqrt(v + eps)

def _scatter_add(tgt, idx, src, axis=0):
    return tgt.at[idx].add(src)

def _segment_sum(src, seg, n):
    return jax.ops.segment_sum(src, seg, n)

class _Rng:

    def __init__(self, key):
        self._k = key

    def _next(self):
        self._k, sub = jax.random.split(self._k)
        return sub

    def normal(self, shape):
        return jax.random.normal(self._next(), shape, dtype=jnp.bfloat16)

    def randint(self, lo, hi, shape):
        return jax.random.randint(self._next(), shape, lo, hi, dtype=jnp.int32)

    def uniform(self, shape, lo=0.0, hi=1.0):
        return jax.random.uniform(self._next(), shape, jnp.bfloat16, lo, hi)

    def permutation(self, n):
        return jax.random.permutation(self._next(), n)
kernel_name = 'adaLN_cond__grouped_kv_mqa__swiglu_ffn__prompt'

def setup_inputs():
    _rng = _Rng(jax.random.key(int.from_bytes(__import__("os").urandom(4), "little")))
    _w = lambda a: (lambda t: t.astype(jnp.bfloat16) if jnp.issubdtype(t.dtype, jnp.floating) else t)(jnp.asarray(a))

    def _A_setup():
        B, S, D, H = (1, 2048, 576, 32)
        Dh = D // H
        return {'x': _w((lambda *s: _rng.normal(s) * 0.05)(B, S, D)), 'wq': _w((lambda *s: _rng.normal(s) * 0.05)(D, H * Dh)), 'wk': _w((lambda *s: _rng.normal(s) * 0.05)(D, Dh)), 'wv': _w((lambda *s: _rng.normal(s) * 0.05)(D, Dh)), 'wo': _w((lambda *s: _rng.normal(s) * 0.05)(H * Dh, D))}
    _A_in = _A_setup()

    def _B_setup():
        B, S, D, F = (1, 2048, 576, 4608)
        return {'x': _w((lambda *s: _rng.normal(s) * 0.05)(B, S, D)), 'w_gate': _w((lambda *s: _rng.normal(s) * 0.05)(D, F)), 'w_up': _w((lambda *s: _rng.normal(s) * 0.05)(D, F)), 'w_down': _w((lambda *s: _rng.normal(s) * 0.05)(F, D))}
    _B_in = _B_setup()
    return {'A_x': _A_in['x'], 'A_wq': _A_in['wq'], 'A_wk': _A_in['wk'], 'A_wv': _A_in['wv'], 'A_wo': _A_in['wo'], 'B_x': _B_in['x'], 'B_w_gate': _B_in['w_gate'], 'B_w_up': _B_in['w_up'], 'B_w_down': _B_in['w_down'], 'c': _w((lambda *s: _rng.normal(s) * 0.05)(1, 576) * 8.0), 'w_mod': _w((lambda *s: _rng.normal(s) * 0.05)(576, 6 * 576) * 576 ** (-0.5) * 8.0)}

def reference(A_x, A_wq, A_wk, A_wv, A_wo, B_x, B_w_gate, B_w_up, B_w_down, c, w_mod):

    def _A_ref(x, wq, wk, wv, wo):
        B, S, D = x.shape
        H = 32
        Dh = D // H
        q = (lambda x, *d: x.transpose(*d))((x @ wq).reshape(B, S, H, Dh), 0, 2, 1, 3)
        k = x @ wk
        v = x @ wv
        scores = jnp.einsum('bhqd,bkd->bhqk', q, k) * Dh ** (-0.5)
        p = _softmax(scores, axis=-1)
        o = jnp.einsum('bhqk,bkd->bhqd', p, v)
        return (lambda x, *d: x.transpose(*d))(o, 0, 2, 1, 3).reshape(B, S, H * Dh) @ wo

    def _B_ref(x, w_gate, w_up, w_down):
        g = _silu(x @ w_gate)
        u = x @ w_up
        return g * u @ w_down
    x = A_x
    mod = (_silu(c) @ w_mod).reshape(c.shape[0], 6, 1, -1)
    sa, ca, ga, sb, cb, gb = (mod[:, 0].copy(), mod[:, 1].copy(), mod[:, 2].copy(), mod[:, 3].copy(), mod[:, 4].copy(), mod[:, 5].copy())
    h = _layernorm(x, axis=-1) * (1 + ca) + sa
    x = x + ga * _A_ref(h, A_wq, A_wk, A_wv, A_wo)
    h = _layernorm(x, axis=-1) * (1 + cb) + sb
    x = x + gb * _B_ref(h, B_w_gate, B_w_up, B_w_down)
    return x
```

```python
import math

import jax
import jax.numpy as jnp
from jax import lax
import jax.experimental.pallas as pl
import jax.experimental.pallas.tpu as pltpu

_H = 32
_EPS = 1e-5
_TQ = 512
_CK = 128
_CF = 512
_UH = 2
_UF = 3

_BF = jnp.bfloat16
_F32 = jnp.float32
_U32 = jnp.uint32


def _mm(a, b):
    return lax.dot_general(a, b, (((1,), (0,)), ((), ())), preferred_element_type=_F32)


def _mm_nt(a, b):
    return lax.dot_general(a, b, (((1,), (1,)), ((), ())), preferred_element_type=_F32)


def _tile_lanes(col, width):
    return jnp.concatenate([col] * (width // 128), axis=1)


def _ln_mod(x, scale1, shift):
    d = x.shape[0]
    mean = jnp.sum(x, axis=0, keepdims=True) * (1.0 / d)
    xc = x - mean
    var = jnp.sum(xc * xc, axis=0, keepdims=True) * (1.0 / d)
    return xc * lax.rsqrt(var + _EPS) * scale1 + shift


def _kernel(xt_hbm, wq_hbm, wkt_hbm, wvt_hbm, wo_hbm, wg_hbm, wu_hbm, wdt_hbm, c_hbm, wmod_hbm,
            out_hbm,
            xt, wq, wkt, wvt, wo, wg, wu, wdt, cv, wmod,
            modc, wqt, wot, q_s, k_s, vt_s, s_s, o_s, x1_s, h2_s, acc_s, out_s,
            sem_in, sem_x, sem_out):
    D, S = xt_hbm.shape
    F = wg_hbm.shape[1]
    DH = D // _H
    NB = S // _TQ
    NC = F // _CF
    NL = _TQ // 128
    PR = DH // 2
    M1 = 2 * D

    cp_c = pltpu.make_async_copy(c_hbm, cv, sem_in.at[0])
    cp_m1 = pltpu.make_async_copy(wmod_hbm.at[:, pl.ds(0, M1)], wmod.at[:, pl.ds(0, M1)], sem_in.at[1])
    cp_wk = pltpu.make_async_copy(wkt_hbm, wkt, sem_in.at[2])
    cp_wv = pltpu.make_async_copy(wvt_hbm, wvt, sem_in.at[3])
    cp_wq = pltpu.make_async_copy(wq_hbm, wq, sem_in.at[4])
    cp_m2 = pltpu.make_async_copy(wmod_hbm.at[:, pl.ds(M1, 6 * D - M1)],
                                  wmod.at[:, pl.ds(M1, 6 * D - M1)], sem_in.at[5])
    cp_wo = pltpu.make_async_copy(wo_hbm, wo, sem_in.at[6])
    cp_x = [pltpu.make_async_copy(xt_hbm.at[:, pl.ds(b * _TQ, _TQ)], xt.at[b], sem_x.at[b])
            for b in range(NB)]
    cp_w = []
    for j in range(NC):
        cols = pl.ds(j * _CF, _CF)
        cp_w.append(pltpu.make_async_copy(wg_hbm.at[:, cols], wg.at[j], sem_in.at[7]))
        cp_w.append(pltpu.make_async_copy(wu_hbm.at[:, cols], wu.at[j], sem_in.at[7]))
        cp_w.append(pltpu.make_async_copy(wdt_hbm.at[:, cols], wdt.at[j], sem_in.at[7]))

    cp_c.start()
    cp_m1.start()
    cp_wq.start()
    cp_wk.start()
    cp_wv.start()
    for cp in cp_x:
        cp.start()

    cp_c.wait()
    cf = cv[...].astype(_F32)
    sc = jnp.broadcast_to((cf * jax.nn.sigmoid(cf)).astype(_BF).astype(_F32), (8, D))

    def mod_cols(lo, hi):
        row = _mm(sc, wmod[:, lo:hi])[0:1, :]
        modc[lo:hi, :] = jnp.broadcast_to(row, (128, hi - lo)).T

    cp_m1.wait()
    mod_cols(0, M1)

    cp_wq.wait()
    wqt[...] = wq[...].astype(_F32).T.astype(_BF)
    cp_wk.wait()
    cp_wv.wait()
    zpad = jnp.zeros((24 - DH, D), _F32)
    wkv = jnp.concatenate([wkt[...].astype(_F32), zpad, wvt[...].astype(_F32), zpad], axis=0)

    qscale = DH ** -0.5 * math.log2(math.e)
    for b in range(NB):
        cp_x[b].wait()
        h = _ln_mod(xt[b].astype(_F32),
                    _tile_lanes(1.0 + modc[D:2 * D, :], _TQ),
                    _tile_lanes(modc[0:D, :], _TQ)).astype(_BF)
        kv = _mm(wkv, h).astype(_BF).astype(_F32)
        kt = jnp.concatenate([kv[0:24], jnp.zeros((128 - 24, _TQ), _F32)], axis=0)
        k_s[b * _TQ:(b + 1) * _TQ, :] = kt.T[:, 0:32]
        rows = lax.broadcasted_iota(jnp.int32, (24, _TQ), 0)
        vt_s[:, b * _TQ:(b + 1) * _TQ] = jnp.where(rows < DH, kv[24:48], 1.0)
        q = pltpu.bitcast((_mm(wqt[...], h) * qscale).astype(_BF), _U32)
        for l in range(NL):
            q_s[b * NL + l, 0:D // 2, :] = q[:, l * 128:(l + 1) * 128]
            q_s[b * NL + l, D // 2:D // 2 + 8, :] = jnp.zeros((8, 128), _U32)

    cp_m2.start()
    cp_wo.start()
    for cp in cp_w:
        cp.start()

    nck = S // _CK

    def load_q(t):
        b = t // _H
        r = (t % _H) * PR
        return pltpu.bitcast(
            jnp.concatenate([q_s[b * NL + l, pl.ds(r, 16), :] for l in range(NL)], axis=1), _BF)

    def pass1(q, slot, c, m8):
        s = _mm(k_s[c * _CK:(c + 1) * _CK, :], q)
        s_s[slot, c * _CK:(c + 1) * _CK, :] = s
        mc = jnp.max(s.reshape(_CK // 8, 8, _TQ), axis=0)
        return mc if m8 is None else jnp.maximum(m8, mc)

    def pass2(slot, c, m, acc):
        p = jnp.exp2(s_s[slot, c * _CK:(c + 1) * _CK, :] - m).astype(_BF)
        r = _mm(vt_s[:, c * _CK:(c + 1) * _CK], p)
        return r if acc is None else acc + r

    def finish(t, acc):
        b = t // _H
        r = (t % _H) * PR
        o = acc / acc[DH:DH + 1, :]
        o = jnp.concatenate([o, jnp.zeros((8, _TQ), _F32)], axis=0)
        o = pltpu.bitcast(o.astype(_BF), _U32)
        for l in range(NL):
            o_s[b * NL + l, pl.ds(r, 16), :] = o[:, l * 128:(l + 1) * 128]

    def step(t, slot, m, with_next):
        m8 = acc = None
        if with_next:
            q = load_q(t + 1)
        for c in range(nck):
            if with_next:
                m8 = pass1(q, 1 - slot, c, m8)
            acc = pass2(slot, c, m, acc)
        finish(t, acc)
        return jnp.max(m8, axis=0, keepdims=True) if with_next else None

    m8 = None
    q0 = load_q(0)
    for c in range(nck):
        m8 = pass1(q0, 0, c, m8)
    m = jnp.max(m8, axis=0, keepdims=True)

    n_steps = NB * _H

    def attn_body(i, m):
        for u in range(_UH):
            m = step(i * _UH + u, u % 2, m, True)
        return m

    n_loop = (n_steps - 1) // _UH
    m = lax.fori_loop(0, n_loop, attn_body, m)
    for t in range(n_loop * _UH, n_steps):
        m = step(t, t % 2, m, t + 1 < n_steps)

    cp_m2.wait()
    mod_cols(M1, 6 * D)
    cp_wo.wait()
    wot[...] = wo[...].astype(_F32).T.astype(_BF)
    for b in range(NB):
        o = pltpu.bitcast(
            jnp.concatenate([o_s[b * NL + l, 0:D // 2, :] for l in range(NL)], axis=1), _BF)
        x1 = xt[b].astype(_F32) + _tile_lanes(modc[2 * D:3 * D, :], _TQ) * _mm(wot[...], o)
        x1_s[b] = x1
        h2 = _ln_mod(x1,
                     _tile_lanes(1.0 + modc[4 * D:5 * D, :], _TQ),
                     _tile_lanes(modc[3 * D:4 * D, :], _TQ))
        h2_s[b] = h2.T.astype(_BF)

    for cp in cp_w:
        cp.wait()

    def out_copy(b):
        return pltpu.make_async_copy(
            out_s.at[b], out_hbm.at[:, pl.ds(pl.multiple_of(b * _TQ, _TQ), _TQ)], sem_out.at[b])

    def ffn_block(b, _):
        acc_s[...] = jnp.zeros(acc_s.shape, _F32)

        def ffn_chunks(i, _):
            for u in range(_UF):
                j = i * _UF + u
                g = _mm(h2_s[b], wg[j])
                up = _mm(h2_s[b], wu[j])
                a = (g * jax.nn.sigmoid(g) * up).astype(_BF)
                acc_s[...] += _mm_nt(wdt[j], a)

        lax.fori_loop(0, NC // _UF, ffn_chunks, None)
        out_s[b] = (x1_s[b] + _tile_lanes(modc[5 * D:6 * D, :], _TQ) * acc_s[...]).astype(out_s.dtype)
        out_copy(b).start()

    lax.fori_loop(0, NB, ffn_block, None)
    for b in range(NB):
        out_copy(b).wait()


@jax.jit
def pallas_adaLN_cond__grouped_kv_mqa__swiglu_ffn__prompt_kernel(
    A_x: jax.Array,
    A_wq: jax.Array,
    A_wk: jax.Array,
    A_wv: jax.Array,
    A_wo: jax.Array,
    B_x: jax.Array,
    B_w_gate: jax.Array,
    B_w_up: jax.Array,
    B_w_down: jax.Array,
    c: jax.Array,
    w_mod: jax.Array,
):
    del B_x
    _, S, D = A_x.shape
    F = B_w_gate.shape[1]
    DH = D // _H
    NB = S // _TQ
    NC = F // _CF
    dt = A_x.dtype
    hbm = pl.BlockSpec(memory_space=pltpu.HBM)
    vm = pltpu.VMEM
    out_t = pl.pallas_call(
        _kernel,
        out_shape=jax.ShapeDtypeStruct((D, S), dt),
        in_specs=[hbm] * 10,
        out_specs=hbm,
        scratch_shapes=[
            vm((NB, D, _TQ), dt),
            vm((D, D), dt),
            vm((DH, D), dt),
            vm((DH, D), dt),
            vm((D, D), dt),
            vm((NC, D, _CF), dt),
            vm((NC, D, _CF), dt),
            vm((NC, D, _CF), dt),
            vm((1, D), dt),
            vm((D, 6 * D), dt),
            vm((6 * D, 128), _F32),
            vm((D, D), _BF),
            vm((D, D), _BF),
            vm((S // 128, D // 2 + 8, 128), _U32),
            vm((S, 32), _F32),
            vm((24, S), _F32),
            vm((2, S, _TQ), _F32),
            vm((S // 128, D // 2 + 8, 128), _U32),
            vm((NB, D, _TQ), _F32),
            vm((NB, _TQ, D), _BF),
            vm((D, _TQ), _F32),
            vm((NB, D, _TQ), dt),
            pltpu.SemaphoreType.DMA((8,)),
            pltpu.SemaphoreType.DMA((NB,)),
            pltpu.SemaphoreType.DMA((NB,)),
        ],
        compiler_params=pltpu.CompilerParams(vmem_limit_bytes=100 * 2 ** 20),
        name="adaln_mqa_swiglu",
    )(A_x[0].T, A_wq, A_wk.T, A_wv.T, A_wo, B_w_gate, B_w_up, B_w_down.T, c, w_mod)
    return out_t.T[None]
```

```python
import contextlib
import functools
import math

import jax
import jax.numpy as jnp
from jax import lax
import jax.experimental.pallas as pl
import jax.experimental.pallas.tpu as pltpu

_H = 32
_EPS = 1e-5
_TQ = 512
_CK = 128
_CF = 512
_U = 4
_UL = 2
_UF = 3
_NVP = 36
_NV0 = 24
_NV1 = 23
_NR = 9
_DENS = (21, 16, 18, 22)
_ONLY = None
_AA = True
_SCOPES = False
_XS = 1
_AF32 = True
_DMA = 2
_P2 = False
_TAIL = 4
_PV = 2
_FLAGS = None

_BF = jnp.bfloat16
_F32 = jnp.float32
_U32 = jnp.uint32


def _scope(name):
    return jax.named_scope(name) if _SCOPES else contextlib.nullcontext()


def _mm(a, b):
    return lax.dot_general(a, b, (((1,), (0,)), ((), ())), preferred_element_type=_F32)


def _mm_nt(a, b):
    return lax.dot_general(a, b, (((1,), (1,)), ((), ())), preferred_element_type=_F32)


def _pack(x):
    return pltpu.bitcast(x.astype(_BF), _U32)


def _unpack(x):
    return pltpu.bitcast(x, _BF)


def _tile_lanes(col, width):
    return jnp.concatenate([col] * (width // 128), axis=1)


def _tree_sum(xs):
    if len(xs) == 1:
        return xs[0]
    h = (len(xs) + 1) // 2
    return _tree_sum(xs[:h]) + _tree_sum(xs[h:])


def _split(n, parts):
    e = [(i * n + parts // 2) // parts for i in range(parts + 1)]
    return list(zip(e[:-1], e[1:]))


def _ln_stats(x):
    d = x.shape[0]
    mean = jnp.sum(x, axis=0, keepdims=True) * (1.0 / d)
    xc = x - mean
    var = jnp.sum(xc * xc, axis=0, keepdims=True) * (1.0 / d)
    return mean, lax.rsqrt(var + _EPS)


def _kernel(xt_hbm, wq_hbm, wkt_hbm, wvt_hbm, wo_hbm, wg_hbm, wu_hbm, wdt_hbm, c_hbm, wmod_hbm,
            out_hbm,
            xt, modc, wqt, wot, h_s, q_s, k_s, kb_s, vt_s, s_s, m_s, pv_s, o_s, wgu_s, wd_s, zero_s,
            sem_in, sem_x, sem_w, sem_out):
    D, S = xt_hbm.shape
    F = wg_hbm.shape[1]
    dt = xt_hbm.dtype
    DH = D // _H
    NB = S // _TQ
    NC = F // _CF
    NL = _TQ // 128
    HT = _TQ // 2
    HD = D // 2
    DP = q_s.shape[1]
    PR = DH // 2
    M1 = 2 * D
    NP = _NR * NC // _UF
    NKB = kb_s.shape[0]
    NPAIR = _H // (2 * _U)
    nck = S // _CK
    wgu = wgu_s.bitcast(_BF)
    wd = wd_s.bitcast(_BF)
    wbase = [0, 640, 1280, 1920, 2432, 2944, 3584]

    def put_q(t, q):
        n = q.shape[0] // DH
        q = jnp.concatenate([q * (DH ** -0.5 * math.log2(math.e)), jnp.zeros((8, _TQ), _F32)], axis=0)
        for i in range(n):
            q_s[t + i] = q[DH * i:DH * i + DP]

    def never():
        return jnp.full((8, 128), zero_s[0], jnp.int32) > 0

    def head_pair(t4, dt1, slot1, dt2, slot2, n_vpu, pre, extra, last):
        n_pre = 0 if pre is None else pre.shape[0] // 8
        n_mxu = S // 8 - n_vpu - n_pre
        lo = n_vpu + n_pre
        mx = [None] * NL
        st = {}
        if dt1 is not None:
            q = q_s.at[4 * t4 + dt1]
            events = {}
            for n in range(n_vpu * NL):
                events.setdefault((2 * n + 1) * n_mxu // (2 * n_vpu * NL), []).append(("v", n))
            for n in range(n_pre):
                events.setdefault((2 * n + 1) * n_mxu // (2 * n_pre), []).append(("p", n))
            for n in range(len(extra)):
                events.setdefault((2 * n + 1) * n_mxu // (2 * len(extra)), []).append(("x", n))
            mask = never() if extra else None

        def scores(ga, gb):
            rows = slice(8 * (lo + ga), 8 * (lo + gb))
            s = _mm(k_s[rows, :], q[...])
            s_s[slot1, rows, :] = s
            for g in range(ga, gb):
                for l in range(NL):
                    x = s[8 * (g - ga):8 * (g - ga + 1), 128 * l:128 * (l + 1)]
                    mx[l] = x if mx[l] is None else jnp.maximum(mx[l], x)
                for kind, n in events.get(g, []):
                    if kind == "v":
                        l, r = divmod(n, n_vpu)
                        lanes = slice(128 * l, 128 * (l + 1))
                        if r == 0:
                            st["qb"] = [jnp.broadcast_to(q[d:d + 1, lanes], (8, 128)) for d in range(DH)]
                        sv = _tree_sum([kb_s[n_pre + r, d] * st["qb"][d] for d in range(DH)])
                        s_s[slot1, 8 * (n_pre + r):8 * (n_pre + r + 1), lanes] = sv
                        mx[l] = jnp.maximum(mx[l], sv)
                    elif kind == "p":
                        sv = pre[8 * n:8 * (n + 1), :]
                        s_s[slot1, 8 * n:8 * (n + 1), :] = sv
                        for l in range(NL):
                            mx[l] = jnp.maximum(mx[l], sv[:, 128 * l:128 * (l + 1)])
                    else:
                        for i, v in enumerate(extra[n]()[::-_XS]):
                            mx[i % NL] = jnp.where(mask, v, mx[i % NL])

        if dt2 is not None:
            m = jnp.broadcast_to(jnp.max(m_s[slot2], axis=0, keepdims=True), (_CK, _TQ))
        tail = _TAIL if last else 0
        for c, (ga, gb) in enumerate(_split(n_mxu - tail, nck)):
            if dt1 is not None:
                scores(ga, gb)
            elif c % 4 == 0:
                extra[0]()
            if dt2 is not None:
                p = jnp.exp2(s_s[slot2, c * _CK:(c + 1) * _CK, :] - m)
                acc = _mm(vt_s[:, c * _CK:(c + 1) * _CK], p)
                if c > 0:
                    acc = acc + (prev if _PV == 2 else pv_s[zero_s[2 * c] if _PV == 0 else 0])
                prev = acc
                if c < nck - 1 and _PV != 2:
                    pv_s[zero_s[2 * c + 1] if _PV == 0 else 0] = acc
        if dt2 is not None:
            o = acc * (1.0 / acc[DH:DH + 1, :])
            o = _pack(jnp.concatenate([o, jnp.zeros((8, _TQ), _F32)], axis=0))
            for l in range(NL):
                o_s[l, pl.ds(t4 * (4 * PR) + dt2 * PR, 16), :] = o[:, l * 128:(l + 1) * 128]
        if dt1 is not None:
            if tail:
                scores(n_mxu - tail, n_mxu)
            m_s[slot1] = jnp.concatenate(mx, axis=1)

    def attn_block(t4, e, n_vpu, pre_of, extra_of):
        if _ONLY not in (None, 'attn'):
            return
        for u in range(_U):
            head_pair(t4, u + _U, (1 - e) * _U + u, u, e * _U + u, n_vpu, pre_of(u), extra_of(u),
                      u == _U - 1)

    def phase1(wq, wkv_s, wo, wg, wu, wdt, cv_s, wmod):
        wkt, wvt, cv = wkv_s.at[0], wkv_s.at[1], cv_s.at[0]
        cp_c = pltpu.make_async_copy(c_hbm, cv, sem_in.at[0])
        cp_m1 = pltpu.make_async_copy(wmod_hbm.at[:, pl.ds(0, M1)], wmod.at[:, pl.ds(0, M1)], sem_in.at[1])
        cp_wk = pltpu.make_async_copy(wkt_hbm, wkt, sem_in.at[2])
        cp_wv = pltpu.make_async_copy(wvt_hbm, wvt, sem_in.at[3])
        cp_wq = pltpu.make_async_copy(wq_hbm, wq, sem_in.at[4])
        cp_m2 = pltpu.make_async_copy(wmod_hbm.at[:, pl.ds(M1, 6 * D - M1)],
                                      wmod.at[:, pl.ds(M1, 6 * D - M1)], sem_in.at[5])
        cp_wo = pltpu.make_async_copy(wo_hbm, wo, sem_in.at[6])
        cp_x = [pltpu.make_async_copy(xt_hbm.at[:, pl.ds(b * _TQ, _TQ)], xt.at[b], sem_x.at[b])
                for b in range(NB)]

        def cp_w(j):
            cols = pl.ds(pl.multiple_of(j * _CF, _CF), _CF)
            return [pltpu.make_async_copy(wg_hbm.at[:, cols], wg.at[j], sem_w.at[j]),
                    pltpu.make_async_copy(wu_hbm.at[:, cols], wu.at[j], sem_w.at[j]),
                    pltpu.make_async_copy(wdt_hbm.at[:, cols], wdt.at[j], sem_w.at[j])]

        def mod_cols(lo, hi):
            cf = cv[...].astype(_F32)
            sc = jnp.broadcast_to(cf * jax.nn.sigmoid(cf), (8, D))
            row = _mm(sc, wmod[:, lo:hi])[0:1, :]
            col = lax.broadcasted_iota(jnp.int32, row.shape, 1) + lo
            one = ((col >= D) & (col < 2 * D)) | ((col >= 4 * D) & (col < 5 * D))
            row = jnp.where(one, row + 1.0, row)
            row = row * jnp.where(col >= 5 * D, 2.0, jnp.where(col >= 3 * D, 0.5, 1.0))
            modc[lo:hi, :] = jnp.broadcast_to(row, (128, hi - lo)).T

        def weight_item(j, i):
            def rows(ref, base):
                x = ref[j, base + 16 * i:base + 16 * (i + 1), :].astype(_F32)
                return [x[:, 128 * t:128 * (t + 1)] for t in range(4)]

            def put(ref, row, lane, val):
                idx = (slice(row, row + 16), slice(128 * lane, 128 * (lane + 1)))
                ref[idx] = val.astype(_BF)
                return pltpu.bitcast(ref[idx], _F32)

            def main_part(w, ref, r0):
                top, bot = rows(ref, r0), rows(ref, 256 + r0)
                sums = [[b11 + b22, b11, b12 - b22, b21 - b11, b22, b11 + b12, b21 + b22]
                        for b11, b12, b21, b22
                        in ((top[t], top[t + 2], bot[t], bot[t + 2]) for t in range(2))]
                out = []
                for p, (va, vb) in enumerate(zip(*sums)):
                    if p in (3, 4, 6):
                        out += [(wbase[p] + r0, va), (wbase[p] + 256 + r0, vb)]
                    elif r0 < 128:
                        out += [(wbase[p] + 256 + r0, va), (wbase[p] + 384 + r0, vb)]
                    elif r0 == 128:
                        out += [(wbase[p] + 128, va), (wbase[p] + 512, vb)]
                    else:
                        out += [(wbase[p], vb), (wbase[p] + 192, va - vb)]
                return [put(wgu.at[j], r + 16 * i, w, v) for r, v in out]

            def rest_part(w, ref):
                r = rows(ref, 512)
                out = []
                for p, va, vb in ((0, r[0], r[1]), (1, r[0], r[1]), (2, r[2], r[3]),
                                  (5, r[0] + r[2], r[1] + r[3])):
                    out += [(wbase[p] + 64, va), (wbase[p] + 576, vb - va)]
                return [put(wgu.at[j], r + 16 * i, w, v) for r, v in out]

            def down_part(g):
                top = wdt[j, 16 * g:16 * (g + 1), :].astype(_F32)
                bot = wdt[j, HD + 16 * g:HD + 16 * (g + 1), :].astype(_F32)
                a11, a12, a21, a22 = top[:, :256], top[:, 256:], bot[:, :256], bot[:, 256:]
                sums = (a11 + a22, a21 + a22, a11, a22, a11 + a12, a21 - a11, a12 - a22)
                return [put(wd.at[j], p * HD + 16 * g, t, v[:, 128 * t:128 * (t + 1)])
                        for p, v in enumerate(sums) for t in range(2)]

            thunks = []
            for w, ref in enumerate((wg, wu)):
                for r0 in (0, 64, 128, 192):
                    thunks.append(functools.partial(main_part, w, ref, r0))
                thunks.append(functools.partial(rest_part, w, ref))
            for g in range(*_split(HD // 16, 4)[i]):
                thunks.append(functools.partial(down_part, g))
            return thunks

        with _scope("p0_mod"):
            cp_wq.start()
            cp_c.start()
            cp_wk.start()
            cp_wv.start()
            cp_x[0].start()
            cp_m1.start()
            for i in range(zero_s.shape[0]):
                zero_s[i] = 0
            cp_wq.wait()
            cp_x[1].start()
            wqt[...] = _pack(wq[...].astype(_F32).T)
            cp_x[0].wait()
            stats0 = _ln_stats(xt[0].astype(_F32))
            if _DMA == 0:
                for cp in cp_x[2:]:
                    cp.start()
            cp_wk.wait()
            cp_wv.wait()
            cp_c.wait()
            cp_m1.wait()
            if _DMA > 0:
                for cp in cp_x[2:]:
                    cp.start()
            mod_cols(0, M1)

        hb = h_s.bitcast(_BF)

        def modulate(b, stats=None):
            x = xt[b].astype(_F32)
            mean, rstd = stats or _ln_stats(x)
            hb.at[b][...] = ((x - mean) * rstd * _tile_lanes(modc[D:2 * D, :], _TQ)
                             + _tile_lanes(modc[0:D, :], _TQ)).astype(_BF)
            return [pltpu.bitcast(hb.at[b][16 * i:16 * (i + 1), 128 * l:128 * (l + 1)], _U32)
                    for l in range(NL) for i in range(D // 16)]

        def keys_values(b):
            zpad = jnp.zeros((DP - DH, D), _F32)
            wkv = jnp.concatenate([wkt[...].astype(_F32), zpad, wvt[...].astype(_F32), zpad], axis=0)
            kv = _mm(wkv, hb[b])
            kt = jnp.concatenate([kv[0:DP], jnp.zeros((128 - DP, _TQ), _F32)], axis=0)
            kk = kt.T[:, 0:DP]
            k_s[b * _TQ:(b + 1) * _TQ, :] = kk
            lo, hi = b * _TQ, min((b + 1) * _TQ, 8 * NKB)
            if hi > lo:
                for d in range(DH):
                    kb_s[lo // 8:hi // 8, d] = jnp.broadcast_to(
                        kk[0:hi - lo, d:d + 1], (hi - lo, 128)).reshape((hi - lo) // 8, 8, 128)
            rows = lax.broadcasted_iota(jnp.int32, (DP, _TQ), 0)
            vt_s[:, b * _TQ:(b + 1) * _TQ] = jnp.where(rows < DH, kv[DP:], 1.0)

        def queries(b, pull):
            mask = never()
            for g, (lo, hi) in enumerate(_split(len(pull), 4)):
                w = [[wqt[4 * DH * g + 8 * i:4 * DH * g + 8 * (i + 1), 128 * k:min(128 * (k + 1), D)]
                      for k in range(5)] for i in range(DH // 2)]
                for n, (x, y) in enumerate(_split(hi - lo, 2 * DH)):
                    w[n // 4][n % 4] = jnp.where(
                        mask, functools.reduce(jnp.bitwise_or, pull[lo + x:lo + y]), w[n // 4][n % 4])
                w = jnp.concatenate([jnp.concatenate(r, axis=1) for r in w], axis=0)
                put_q(b * _H + 8 * g, _mm(_unpack(w), hb[b]))

        with _scope("p1_q0"):
            cp_x[1].wait()
            if _DMA == 2:
                for cp in cp_w(0):
                    cp.start()
            modulate(0, stats0)
            keys_values(0)
            queries(0, modulate(1))
        with _scope("p1b_q1"):
            for b in range(2, NB):
                cp_x[b].wait()
            for cp in (cp_w(0) if _DMA < 2 else []) + [cp_wo, cp_m2]:
                cp.start()
            keys_values(1)
            queries(1, [v for b in range(2, NB) for v in modulate(b)])
            for b in range(2, NB):
                keys_values(b)

        with _scope("p2_first"):
            def first(u):
                extra = [t for i in range(*_split(4, _U)[u]) for t in weight_item(0, i)]
                more = []
                if u == _U - 2:
                    wot[...] = _pack(wo[...].astype(_F32).T)
                    more = [lambda i=i, k=k: [pltpu.bitcast(wot[i:i + 8, k:k + 128], _F32)]
                            for k in range(0, 512, 128) for i in range(32, HD, 64)]
                if u == _U - 1:
                    more = [lambda k=k: mod_cols(k, k + 128) or [] for k in range(M1, 6 * D, 128)]
                both = [((2 * i + 1) / len(t), f) for t in (extra, more) for i, f in enumerate(t)]
                extra = [f for _, f in sorted(both, key=lambda e: e[0])]
                head_pair(0, u, u, None, None, _NVP, None, extra, False)

            for cp in cp_w(0):
                cp.wait()
            for cp in cp_w(1):
                cp.start()
            for u in range(_U):
                if u == _U - 2:
                    cp_wo.wait()
                if u == _U - 1:
                    cp_m2.wait()
                first(u) if _P2 else pl.when(zero_s[3 + u] == 0)(functools.partial(first, u))

        def first_block(t4, e):
            for cp in cp_w(t4 + 1):
                cp.wait()

            @pl.when(t4 + 2 < NC)
            def _():
                for cp in cp_w(t4 + 2):
                    cp.start()

            pl.when(zero_s[1 + e] == 0)(functools.partial(
                attn_block, t4, e, _NV0, lambda u: None, functools.partial(weight_item, t4 + 1)))

        def first_pair(i, _):
            first_block(2 * i, 0)
            first_block(2 * i + 1, 1)

        with _scope("p3_attn0"):
            first_pair(0, None)
            lax.fori_loop(1, NPAIR, first_pair, None)

    vm = pltpu.VMEM
    pl.run_scoped(phase1, vm((D, D), dt), vm((8, DH, D), dt), vm((D, D), dt), vm((NC, D, _CF), dt),
                  vm((NC, D, _CF), dt), vm((NC, D, _CF), dt), vm((32, 1, D), dt), vm((D, 6 * D), dt))

    def phase2(qp_s, pre_s, x1_s, h2_s, acc_s, out_s):
        def heads(b, lo, hi):
            return _unpack(jnp.concatenate(
                [o_s[l, pl.ds(pl.multiple_of(b * HD + lo // 2, 8), (hi - lo) // 2), :]
                 for l in range(NL)], axis=1))

        def second_norm(b, attn, filler):
            x1 = xt[b].astype(_F32) + _tile_lanes(modc[2 * D:3 * D, :], _TQ) * attn
            x1_s[...] = x1
            filler()
            mean, rstd = _ln_stats(x1)
            h2 = (x1 - mean) * rstd * _tile_lanes(modc[4 * D:5 * D, :], _TQ) + _tile_lanes(modc[3 * D:4 * D, :], _TQ)
            a11, a12, r1 = h2[0:256, :HT], h2[256:512, :HT], h2[512:D, :HT]
            a21, a22, r2 = h2[0:256, HT:], h2[256:512, HT:], h2[512:D, HT:]
            tiles = []
            for a, r in ((a11 + a22, r1), (a21 + a22, r2), (a11, r1), (a22, None), (a11 + a12, None),
                         (a21 - a11, r2 - r1), (a12 - a22, None)):
                if r is None:
                    tiles.append(a)
                else:
                    tiles += [a[128:256], a[0:128], a[128:192], r, a[192:256], r]
            h2_s[...] = _pack(jnp.concatenate(tiles, axis=0).T)

        def ffn_iter(j0, count, fresh, it=None):
            pre = it is not None
            hbase = [0, 4, 8, 12, 14, 16, 20]
            total = _UF * (9 * _DENS[0] + 7 * _DENS[1] + 2 * _DENS[2] + 5 * _DENS[3])
            st = dict(done=0, weight=0)
            mask = never()

            def chain():
                i, n = divmod(st["done"], _H * NL)
                st["done"] += 1
                if n == 0:
                    st["kb"] = [kb_s[it * _NR + i, d] for d in range(DH)]
                h, l = divmod(n, NL)
                lanes = slice(128 * l, 128 * (l + 1))
                sv = _tree_sum([
                    st["kb"][d] * jnp.broadcast_to(qp_s[h * DP + d:h * DP + d + 1, lanes], (8, 128))
                    for d in range(DH)])
                pre_s[h, pl.ds(pl.multiple_of((it * _NR + i) * 8, 8), 8), lanes] = sv
                return sv

            def tie(tiles, weight, pull):
                nr = tiles[0].shape[0] // 8
                rows = [[x[8 * i:8 * (i + 1)] for i in range(nr)] for x in tiles]
                used = [0] * nr

                def attach(i, v):
                    while used[i] == len(tiles):
                        i = (i + 1) % nr
                    rows[used[i]][i] = jnp.where(mask, pltpu.bitcast(v, _U32), rows[used[i]][i])
                    used[i] += 1

                if pre:
                    st["weight"] += weight
                    n = _H * NL * _NR * st["weight"] // total - st["done"]
                    for k in range(n):
                        attach((2 * k + 1) * nr // (2 * n), chain())
                if pull is not None and _AA:
                    n = pull.shape[0] // 8
                    for k in range(n):
                        attach(k * nr // n, pull[8 * k:8 * (k + 1)])
                return [jnp.concatenate(r, axis=0) for r in rows]

            def proj(j, w, finish):
                dens = _DENS[w]
                out = []

                def wt(p, i, n):
                    return wgu[j, wbase[p] + 128 * i:wbase[p] + 128 * (i + n), 128 * w:128 * (w + 1)]

                def ht(p, i):
                    return h2_s[:, 128 * (hbase[p] + i):128 * (hbase[p] + i + 1)]

                long = (1, 2, 0, 5)
                hs = tie([ht(p, 3) for p in long], _DENS[0], None)
                sh = {p: _mm(_unpack(x), wt(p, 0, 1)) for p, x in zip(long, hs)}

                def two(*pts):
                    hs = tie([ht(p, k + (t if p in long else 0)) for p, t in pts for k in range(2)],
                             dens, out[-1] if w and out else None)
                    ms = []
                    for n, (p, t) in enumerate(pts):
                        m = _mm(_unpack(jnp.concatenate(hs[2 * n:2 * n + 2], axis=1)),
                                wt(p, 2 * t + (p in long), 2))
                        ms.append(m + sh[p] if p in long else m)
                    return ms

                keep = []
                for t in range(2):
                    m2, m4 = two((1, t), (3, t))
                    out.append(finish(len(out), m2 + m4))
                    keep.append((m2, m4))
                for t in range(2):
                    m3, m5 = two((2, t), (4, t))
                    out.append(finish(len(out), m3 + m5))
                    keep[t] = (m3 - keep[t][0], keep[t][1] - m5)
                for t in range(2):
                    m1, m7 = two((0, t), (6, t))
                    out.append(finish(len(out), (keep[t][1] + m1) + m7))
                    keep[t] = keep[t][0] + m1
                for t, m6 in enumerate(two((5, 0), (5, 1))):
                    out.append(finish(len(out), keep[t] + m6))
                return out

            for dj in range(count):
                j = j0 + dj
                g = proj(j, 0, lambda n, x: x)
                a = proj(j, 1, lambda n, u: (g[n] * u) * (1.0 + jnp.tanh(g[n])))
                b12, b21, b11, b22 = [jnp.concatenate(a[2 * n:2 * n + 2], axis=1) for n in range(4)]
                for n, (p, x) in enumerate(((1, b11), (3, b21 - b11), (5, b11 + b12), (4, b22),
                                            (0, b11 + b22), (2, b12 - b22), (6, b21 + b22))):
                    w = pltpu.bitcast(wd[j, p * HD:(p + 1) * HD, :], _U32)
                    ws = tie([w[:, :128], w[:, 128:]] * (2 if n < 2 and _AA else 1),
                             _DENS[2 if n < 2 else 3], a[6 + n] if n < 2 else None)
                    x = x if _AF32 else x.astype(_BF)
                    if len(ws) == 2:
                        y = _mm_nt(_unpack(jnp.concatenate(ws, axis=1)), x)
                    else:
                        y = jnp.concatenate([
                            _mm_nt(_unpack(jnp.concatenate(ws[2 * t:2 * t + 2], axis=1)),
                                   x[128 * t:128 * (t + 1)]) for t in range(2)], axis=1)
                    if dj > 0 or fresh is False:
                        y = y + acc_s[p]
                    elif fresh is not True:
                        y = y + jnp.where(fresh, 0.0, acc_s[p])
                    acc_s[p] = y

        def out_copy(b):
            return pltpu.make_async_copy(
                out_s.at[b], out_hbm.at[:, pl.ds(pl.multiple_of(b * _TQ, _TQ), _TQ)], sem_out.at[b])


        def ffn_result(b):
            m1, m2, m3, m4, m5, m6, m7 = [acc_s[p] for p in range(7)]
            y = jnp.concatenate([
                jnp.concatenate([m1 + m4 - m5 + m7, m3 + m5], axis=1),
                jnp.concatenate([m2 + m4, m1 - m2 + m3 + m6], axis=1)], axis=0)
            out_s[b] = (x1_s[...] + _tile_lanes(modc[5 * D:6 * D, :], _TQ) * y).astype(dt)

        def token_block(b, _):
            def later_queries():
                for i in range(3):
                    g8 = jnp.minimum(3 * b + i, 7)
                    w = wqt[pl.ds(pl.multiple_of((g8 & 3) * (4 * DH), 8), 4 * DH), :]
                    put_q(2 * _H + 8 * g8,
                          _mm(_unpack(w), h_s.bitcast(_BF)[lax.shift_right_logical(g8, 2) + 2]))

            with _scope("p5_oproj"):
                for i in range(_H // 2 - _U):
                    qp_s[i * DP:(i + 1) * DP, :] = q_s[(b + 1) * _H + _U + i]
                second_norm(b, _mm(_unpack(wot[...]), heads(b, 0, D)), later_queries)
                for i in range(_H // 2 - _U, _H):
                    qp_s[i * DP:(i + 1) * DP, :] = q_s[jnp.minimum((b + 1) * _H + _U + i, NB * _H - 1)]
            with _scope("p6_ffn"):
                if _ONLY in (None, "ffn"):
                    lax.fori_loop(0, NC // _UF, lambda i, _: ffn_iter(i * _UF, _UF, i == 0, i), None)
                ffn_result(b)
                out_copy(b).start()
            with _scope("p7_attn"):
                def block(i, e):
                    attn_block(2 * ((b + 1) * NPAIR + i) + e, e, _NV1,
                               lambda u: pre_s.at[(2 * i + e) * _U + u], lambda u: [])

                def pair(i, _):
                    block(i, 0)
                    pl.when((b + 1) * NPAIR + i < NB * NPAIR - 1)(functools.partial(block, i, 1))

                lax.fori_loop(0, NPAIR, pair, None)

        lax.fori_loop(0, NB - 1, token_block, None)
        with _scope("p8_last"):
            KD = 384
            early = heads(NB - 1, 0, KD)
            parts = []
            pieces = _split(D // 16, _U * 4)

            def wo_piece():
                a, b = pieces[len(parts)]
                parts.append(_mm(_unpack(wot[8 * a:8 * b, 0:KD]), early))

            for u in range(_U):
                head_pair(0, None, None, NB * _H - _U + u, _U + u, 0, None, [wo_piece], False)
            attn = jnp.concatenate(parts, axis=0) + _mm(_unpack(wot[:, KD:D]), heads(NB - 1, KD, D))
            second_norm(NB - 1, attn, lambda: None)
            ffn_iter(0, 1, True)
        with _scope("p9_ffn"):
            if _ONLY in (None, "ffn"):
                lax.fori_loop(0, (NC - 1) // _UL, lambda i, _: ffn_iter(1 + i * _UL, _UL, False), None)
            ffn_result(NB - 1)
            out_copy(NB - 1).start()
            for b in range(NB):
                out_copy(b).wait()

    pl.run_scoped(phase2, vm((_H * DP, _TQ), _F32), vm((_H, 8 * NP, _TQ), _F32), vm((D, _TQ), _F32),
                  vm((HT // 2, 22 * 128), _U32), vm((7, HD, HT), _F32), vm((NB, D, _TQ), dt))


@jax.jit
def pallas_adaLN_cond__grouped_kv_mqa__swiglu_ffn__prompt_kernel(
    A_x: jax.Array,
    A_wq: jax.Array,
    A_wk: jax.Array,
    A_wv: jax.Array,
    A_wo: jax.Array,
    B_x: jax.Array,
    B_w_gate: jax.Array,
    B_w_up: jax.Array,
    B_w_down: jax.Array,
    c: jax.Array,
    w_mod: jax.Array,
):
    del B_x
    _, S, D = A_x.shape
    F = B_w_gate.shape[1]
    DH = D // _H
    NB = S // _TQ
    NC = F // _CF
    dt = A_x.dtype
    hbm = pl.BlockSpec(memory_space=pltpu.HBM)
    vm = pltpu.VMEM
    out_t = pl.pallas_call(
        _kernel,
        out_shape=jax.ShapeDtypeStruct((D, S), dt),
        in_specs=[hbm] * 10,
        out_specs=hbm,
        scratch_shapes=[
            vm((NB, D, _TQ), dt),
            vm((6 * D, 128), _F32),
            vm((D // 2, D), _U32),
            vm((D // 2, D), _U32),
            vm((NB, D // 2, _TQ), _U32),
            vm((NB * _H, 24, _TQ), _F32),
            vm((S, 24), _F32),
            vm((max(_NVP, _NV0, _NV1 + _NR * NC // _UF), 20, 8, 128), _F32),
            vm((24, S), _F32),
            vm((2 * _U, S, _TQ), _F32),
            vm((2 * _U, 8, _TQ), _F32),
            vm((1, 24, _TQ), _F32),
            vm((_TQ // 128, NB * D // 2 + 32, 128), _U32),
            vm((NC, 32 * 64, 256), _U32),
            vm((NC, 7 * D // 4, _CF // 2), _U32),
            pltpu.SMEM((32,), jnp.int32),
            pltpu.SemaphoreType.DMA((7,)),
            pltpu.SemaphoreType.DMA((NB,)),
            pltpu.SemaphoreType.DMA((NC,)),
            pltpu.SemaphoreType.DMA((NB,)),
        ],
        compiler_params=pltpu.CompilerParams(vmem_limit_bytes=126 * 2 ** 20, flags=_FLAGS),
        name="adaln_mqa_swiglu",
    )(A_x[0].T, A_wq, A_wk.T, A_wv.T, A_wo, B_w_gate, B_w_up, B_w_down.T, c, w_mod)
    return out_t.T[None]
```

```python
import functools
import math

import jax
import jax.numpy as jnp
from jax import lax
import jax.experimental.pallas as pl
import jax.experimental.pallas.tpu as pltpu

_H = 32
_EPS = 1e-5
_TQ = 512
_CF = 512
_U = 4
_UF = 3
_UL = 2
_NV_FILL = (32, 32, 20, 20)
_NV_FIRST = 36
_NV_LATER = 38
_NV_AHEAD = 28
_SHARE = (22, 24, 24, 22, 20, 20, 16, 16, 20, 24, 16, 16, 16, 14, 12, 4, 9, 18, 15, 15, 15, 24, 24)
_SUM_LO, _SUM_HI = 2.0 ** -30, 2.0 ** 120

_BF = jnp.bfloat16
_F32 = jnp.float32
_U32 = jnp.uint32


def _mm(a, b):
    return lax.dot_general(a, b, (((1,), (0,)), ((), ())), preferred_element_type=_F32)


def _mm_nt(a, b):
    return lax.dot_general(a, b, (((1,), (1,)), ((), ())), preferred_element_type=_F32)


def _pack(x):
    return pltpu.bitcast(x.astype(_BF), _U32)


def _unpack(x):
    return pltpu.bitcast(x, _BF)


def _tile_lanes(col):
    return jnp.concatenate([col] * (_TQ // 128), axis=1)


def _tree_sum(xs):
    if len(xs) == 1:
        return xs[0]
    h = (len(xs) + 1) // 2
    return _tree_sum(xs[:h]) + _tree_sum(xs[h:])


def _split(n, parts):
    e = [(i * n + parts // 2) // parts for i in range(parts + 1)]
    return list(zip(e[:-1], e[1:]))


def _interleave(*lists):
    both = [((2 * i + 1) / len(t), x) for t in lists for i, x in enumerate(t)]
    return [x for _, x in sorted(both, key=lambda e: e[0])]


def _layernorm(x):
    d = x.shape[0]
    xc = x - jnp.sum(x, axis=0, keepdims=True) * (1.0 / d)
    var = jnp.sum(xc * xc, axis=0, keepdims=True) * (1.0 / d)
    return xc * lax.rsqrt(var + _EPS)


def _kernel(xt_hbm, wq_hbm, wkt_hbm, wvt_hbm, wo_hbm, wg_hbm, wu_hbm, wdt_hbm, c_hbm, wmod_hbm,
            out_hbm,
            xt, modc, wqt, wot_s, h_s, q_s, k_s, kb_s, vt_s, p_s, n_s, bad_s, o_s, wgu_s, wd_s,
            zero_s, sem_in, sem_x, sem_w, sem_out):
    D, S = xt_hbm.shape
    F = wg_hbm.shape[1]
    dt = xt_hbm.dtype
    DH = D // _H
    DP = q_s.shape[1]
    HD = D // 2
    HT = _TQ // 2
    NB = S // _TQ
    NC = F // _CF
    NL = _TQ // 128
    NPAIR = _H // (2 * _U)
    hb = h_s.bitcast(_BF)
    wot = wot_s.bitcast(_BF).at[0]
    wgu = wgu_s.bitcast(_BF)
    wd = wd_s.bitcast(_BF)
    wide = (1, 2, 0, 5)
    wbase = [0, 640, 1280, 1920, 2432, 2944, 3584]
    hbase = [0, 4, 8, 12, 14, 16, 20]

    def never():
        return jnp.full((8, 128), zero_s[0], jnp.int32) > 0

    def own_region(i, fn):
        pl.when(zero_s[1 + i] == 0)(fn)

    def put_weights(ref, w):
        w = w.astype(_F32)
        w = jnp.concatenate([w, w[512:D]], axis=0).T
        a, b = w[:HD], w[HD:]
        low = lax.broadcasted_iota(jnp.int32, (HD, 128), 1) < 64
        ref[...] = jnp.concatenate(
            [a[:, 0:384], jnp.where(low, a[:, 384:512], a[:, 384:512] - b[:, 384:512]),
             b[:, 0:384], jnp.where(low, b[:, 384:512], b[:, 512:640] - a[:, 512:640]),
             jnp.where(low, a[:, 512:640], b[:, 384:512])], axis=1).astype(ref.dtype)

    def project(w, x, work):
        mask = never()
        nr = w.shape[0] // 8
        view = _unpack if w.dtype == _U32 else lambda v: v

        def streamed(k, vs):
            rows = [w[8 * i:8 * (i + 1), k:k + 128] for i in range(nr)]
            for i, (a, b) in enumerate(_split(len(vs), nr)):
                if b > a:
                    rows[i] = jnp.where(mask, functools.reduce(jnp.maximum, vs[a:b]), rows[i])
            return view(jnp.concatenate(
                [jnp.concatenate(rows, axis=0), w[:, k + 128:k + 512]], axis=1))

        shared = _mm(view(w[:, 1024:1152]), _unpack(jnp.concatenate([x[256:HD], x[224:256]], axis=0)))
        cols = []
        for l, (lo, hi) in enumerate(_split(len(work), NL)):
            xl, sh = [v[:, 128 * l:128 * (l + 1)] for v in (x, shared)]
            mid = (lo + hi) // 2
            cols.append((
                _mm(streamed(0, work[lo:mid]), _unpack(xl[0:256])) + sh,
                _mm(streamed(512, work[mid:hi]),
                    _unpack(jnp.concatenate([xl[0:224], xl[256:HD]], axis=0))) + sh))
        return [jnp.concatenate(c, axis=1) for c in zip(*cols)]

    def put_q(t, halves):
        for n, q in enumerate(halves):
            heads = q.shape[0] // DH
            q = jnp.concatenate([q, jnp.zeros((8, _TQ), _F32)], axis=0)
            for i in range(heads):
                q_s[t + n * (_H // 2) + i] = q[DH * i:DH * i + DP]

    def put_o(t, l, num):
        o = num * (1.0 / num[DH:DH + 1, :])
        o = _pack(jnp.concatenate([o, jnp.zeros((8, 128), _F32)], axis=0))
        o_s[l, pl.ds(t * (DH // 2), 16), :] = o
        return o

    def vpu_weights(q, lo, hi, l):
        return jnp.exp2(_tree_sum([
            kb_s[lo:hi, d] * jnp.broadcast_to(q[d:d + 1, 128 * l:128 * (l + 1)], (8, 128))
            for d in range(DH)]))

    def attn_step(t, dst, src, n_vpu, n_ahead, ahead, work):
        lo = n_vpu + n_ahead
        n_mxu = S // 8 - lo
        n_rows = n_mxu + (0 if src is None else S // 128 * DP // 8)
        due = {}
        row = [0]
        mask = never()

        def spread(fns):
            for n, fn in enumerate(fns):
                due.setdefault((2 * n + 1) * n_rows // (2 * len(fns)), []).append(fn)

        def tied(x):
            rows = []
            for i in range(0, x.shape[0], 8):
                vs = [v for fn in due.get(row[0], []) for v in fn()]
                row[0] += 1
                rows.append(x[i:i + 8])
                if vs:
                    v = functools.reduce(jnp.maximum, vs)
                    rows[-1] = jnp.where(mask[:, :x.shape[1]], v[:, :x.shape[1]], rows[-1])
            return jnp.concatenate(rows, axis=0)

        def weights(a, b):
            cut = a if ahead is None else min(max(8 * _NV_AHEAD, a), b)
            if cut == a:
                return p_s[src, a:b, :]
            if cut == b:
                return ahead[a:b, :]
            return jnp.concatenate([ahead[a:cut, :].astype(_F32), p_s[src, cut:b, :]], axis=0)

        if t is not None:
            q = q_s.at[t]
            vpu = []
            for l in range(NL):
                p = vpu_weights(q, n_ahead, lo, l)
                p_s[dst, 8 * n_ahead:8 * lo, 128 * l:128 * (l + 1)] = p.reshape(8 * n_vpu, 128)
                vpu += [lambda v=p[r]: [v] for r in range(n_vpu)]
            spread(vpu)
            spread([lambda fn=fn: fn()[-4:] for fn in work])
        num = None
        for c, (a, b) in enumerate(_split(n_mxu, S // 128)):
            if t is not None:
                keys = slice(8 * (lo + a), 8 * (lo + b))
                p_s[dst, keys, :] = jnp.exp2(_mm(tied(k_s[keys, :]), q[...]))
            elif c % 8 == 0:
                work[c // 8]()
            if src is not None:
                r = _mm(tied(vt_s[:, 128 * c:128 * (c + 1)]), weights(128 * c, 128 * (c + 1)))
                num = r if c == 0 else num + r
        return num

    def normalize(t, slot, l):
        lanes = slice(128 * l, 128 * (l + 1))
        num = n_s[slot, :, lanes]
        safe = (num[DH:DH + 1, :] >= _SUM_LO) & functools.reduce(
            jnp.logical_and, [jnp.abs(num[i:i + 8]) <= _SUM_HI for i in range(0, DP, 8)])
        bad = jnp.where(safe, bad_s[:, lanes], 1.0)
        bad_s[:, lanes] = bad
        o = pltpu.bitcast(put_o(t, l, num), _F32)
        return [bad, o[0:8], o[8:16]]

    def attn_block(t, e, n_vpu, n_ahead, ahead_of, work_of, pending):
        for u in range(_U):
            this, other = e * _U + u, (1 - e) * _U + u
            norm = [functools.partial(normalize, t - _U + u, other, l)
                    for l in range(NL if pending else 0)]
            n_s[this] = attn_step(t + _U + u, other, this, n_vpu, n_ahead, ahead_of(u),
                                  _interleave(work_of(u), norm))

    def guarded(b, consume):
        def exact(n, _):
            h = lax.shift_right_logical(n, 2)
            l = n & (NL - 1)
            lanes = pl.ds(pl.multiple_of(128 * l, 128), 128)
            s = _mm(k_s[...], q_s[b * _H + h, :, lanes])
            num = _mm(vt_s[...], jnp.exp2(s - jnp.max(s, axis=0, keepdims=True)))
            n_s[h & (2 * _U - 1), :, lanes] = num
            put_o(b * _H + h, l, num)

        def attempt(state):
            retry = state > 0
            pl.when(retry)(lambda: lax.fori_loop(0, _H * NL, exact, None))
            consume(retry)
            unsafe = jnp.max(bad_s[...]) > 0.0
            bad_s[...] = jnp.zeros(bad_s.shape, _F32)
            return jnp.where(unsafe, state + 1, 2)

        lax.while_loop(lambda state: state < 2, attempt, jnp.int32(0))

    def phase1(wq, wkv_s, wo, wg, wu, wdt, cv_s, wmod):
        wkt, wvt, cv = wkv_s.at[0], wkv_s.at[1], cv_s.at[0]
        cp_c, cp_wk, cp_wv, cp_wq, cp_wo = [
            pltpu.make_async_copy(src, dst, sem_in.at[i]) for i, (src, dst) in enumerate(
                ((c_hbm, cv), (wkt_hbm, wkt), (wvt_hbm, wvt), (wq_hbm, wq), (wo_hbm, wo)))]
        mcut = (0, 512, 2 * D, 6 * D)
        cp_m = [pltpu.make_async_copy(wmod_hbm.at[:, pl.ds(a, b - a)], wmod.at[:, pl.ds(a, b - a)],
                                      sem_in.at[5 + i])
                for i, (a, b) in enumerate(zip(mcut, mcut[1:]))]
        cp_x = [pltpu.make_async_copy(xt_hbm.at[:, pl.ds(b * _TQ, _TQ)], xt.at[b], sem_x.at[b])
                for b in range(NB)]

        def cp_w(j):
            cols = pl.ds(pl.multiple_of(j * _CF, _CF), _CF)
            return [pltpu.make_async_copy(src.at[:, cols], dst.at[j & 1], sem_w.at[j])
                    for src, dst in ((wg_hbm, wg), (wu_hbm, wu), (wdt_hbm, wdt))]

        def start(copies):
            for cp in copies:
                cp.start()

        def wait(copies):
            for cp in copies:
                cp.wait()

        def mod_cols(sc, lo, hi):
            row = _mm(sc, wmod[:, lo:hi])[0:1, :]
            col = lax.broadcasted_iota(jnp.int32, row.shape, 1) + lo
            one = ((col >= D) & (col < 2 * D)) | ((col >= 4 * D) & (col < 5 * D))
            row = jnp.where(one, row + 1.0, row)
            row = row * jnp.where(col >= 5 * D, 2.0, jnp.where(col >= 3 * D, 0.5, 1.0))
            modc[lo:hi, :] = jnp.broadcast_to(row, (128, hi - lo)).T
            return []

        def ffn_weights(j, i):
            def rows(ref, base):
                x = ref[j & 1, base + 16 * i:base + 16 * (i + 1), :].astype(_F32)
                return [x[:, 128 * t:128 * (t + 1)] for t in range(4)]

            def put(ref, row, lane, val):
                idx = (slice(row, row + 16), slice(128 * lane, 128 * (lane + 1)))
                ref[idx] = val.astype(_BF)
                return pltpu.bitcast(ref[idx], _F32)

            def main_part(w, ref, r0):
                top, bot = rows(ref, r0), rows(ref, 256 + r0)
                sums = [[b11 + b22, b11, b12 - b22, b21 - b11, b22, b11 + b12, b21 + b22]
                        for b11, b12, b21, b22
                        in ((top[t], top[t + 2], bot[t], bot[t + 2]) for t in range(2))]
                out = []
                for p, (va, vb) in enumerate(zip(*sums)):
                    if p not in wide:
                        out += [(wbase[p] + r0, va), (wbase[p] + 256 + r0, vb)]
                    elif r0 < 128:
                        out += [(wbase[p] + 256 + r0, va), (wbase[p] + 384 + r0, vb)]
                    elif r0 == 128:
                        out += [(wbase[p] + 128, va), (wbase[p] + 512, vb)]
                    else:
                        out += [(wbase[p], vb), (wbase[p] + 192, va - vb)]
                return [put(wgu.at[j], r + 16 * i, w, v) for r, v in out]

            def rest_part(w, ref):
                r = rows(ref, 512)
                out = []
                for p, va, vb in ((0, r[0], r[1]), (1, r[0], r[1]), (2, r[2], r[3]),
                                  (5, r[0] + r[2], r[1] + r[3])):
                    out += [(wbase[p] + 64, va), (wbase[p] + 576, vb - va)]
                return [put(wgu.at[j], r + 16 * i, w, v) for r, v in out]

            def down_part(g):
                top = wdt[j & 1, 16 * g:16 * (g + 1), :].astype(_F32)
                bot = wdt[j & 1, HD + 16 * g:HD + 16 * (g + 1), :].astype(_F32)
                a11, a12, a21, a22 = top[:, :256], top[:, 256:], bot[:, :256], bot[:, 256:]
                sums = (a11 + a22, a21 + a22, a11, a22, a11 + a12, a21 - a11, a12 - a22)
                return [put(wd.at[j], p * HD + 16 * g, t, v[:, 128 * t:128 * (t + 1)])
                        for p, v in enumerate(sums) for t in range(2)]

            fns = []
            for w, ref in enumerate((wg, wu)):
                fns += [functools.partial(main_part, w, ref, r0) for r0 in (0, 64, 128, 192)]
                fns.append(functools.partial(rest_part, w, ref))
            return fns + [functools.partial(down_part, g) for g in range(*_split(HD // 16, 4)[i])]

        def modulate(b):
            hb.at[b][...] = (_layernorm(xt[b].astype(_F32)) * _tile_lanes(modc[D:2 * D, :])
                             + _tile_lanes(modc[0:D, :])).astype(_BF)
            return [pltpu.bitcast(hb.at[b][16 * i:16 * (i + 1), 128 * l:128 * (l + 1)], _F32)
                    for l in range(NL) for i in range(D // 16)]

        def keys_values(b, centre=None):
            zpad = jnp.zeros((DP - DH, D), _F32)
            wkv = jnp.concatenate([wkt[...].astype(_F32), zpad, wvt[...].astype(_F32), zpad], axis=0)
            kv = _mm(wkv, hb[b])
            kt = kv[0:DP] * (DH ** -0.5 * math.log2(math.e))
            k = jnp.concatenate([kt, jnp.zeros((128 - DP, _TQ), _F32)], axis=0).T[:, 0:DP]
            if centre is None:
                centre = jnp.sum(k, axis=0, keepdims=True) * (1.0 / _TQ)
            k_s[b * _TQ:(b + 1) * _TQ, :] = k - centre
            rows = lax.broadcasted_iota(jnp.int32, (DP, _TQ), 0)
            vt_s[:, b * _TQ:(b + 1) * _TQ] = jnp.where(rows < DH, kv[DP:], 1.0)
            return centre

        def spread_keys(lo, hi):
            k = k_s[8 * lo:8 * hi, :]
            cols = [jnp.broadcast_to(k[:, d:d + 1], (8 * (hi - lo), 128)).reshape(hi - lo, 8, 128)
                    for d in range(DH)]
            for d in range(DH):
                kb_s[lo:hi, d] = cols[d]
            return [lambda c=c: [c[hi - lo - 1]] for c in cols]

        def queries(b, work):
            put_q(b * _H, project(wqt[...], pltpu.bitcast(hb[b], _U32), work))

        start([cp_c, cp_m[0], cp_m[1], cp_wk, cp_wv])
        for i in range(zero_s.shape[0]):
            zero_s[i] = 0
        bad_s[...] = jnp.zeros(bad_s.shape, _F32)
        cp_c.wait()
        cf = cv[...].astype(_F32)
        sc = jnp.broadcast_to(cf * jax.nn.sigmoid(cf), (8, D))
        cp_m[0].wait()
        cp_wq.start()
        mod_cols(sc, mcut[0], mcut[1])
        cp_m[1].wait()
        cp_x[0].start()
        mod_cols(sc, mcut[1], mcut[2])
        cp_wq.wait()
        cp_x[1].start()
        put_weights(wqt, wq[...])

        start(cp_x[2:])
        wait([cp_wk, cp_wv, cp_x[0]])
        modulate(0)
        centre = keys_values(0)
        n_ready = max(_NV_FILL)
        spread_keys(0, n_ready)
        queries(0, [])

        start(cp_w(0))
        wait(cp_x[1:])
        start([cp_wo, cp_m[2]])
        modulate(1)
        keys_values(1, centre)
        queries(1, [v for b in range(2, NB) for v in modulate(b)])
        for b in range(2, NB):
            keys_values(b, centre)

        def fill(u):
            if u < 2:
                more = spread_keys(*(n_ready + x for x in _split(kb_s.shape[0] - n_ready, 2)[u]))
            elif u == 2:
                put_weights(wot, wo[...])
                more = [lambda i=i, k=k: [pltpu.bitcast(wot[i:i + 16, k:k + 128], _F32)]
                        for k in (0, 512, 128, 640, 256, 768, 384, 896, 1024) for i in (112, 240)]
            else:
                more = [functools.partial(mod_cols, sc, k, k + 128) for k in range(2 * D, 6 * D, 128)]
            attn_step(u, u, None, _NV_FILL[u], 0, None, _interleave(ffn_weights(0, u), more))

        start(cp_w(1))
        for u, copies in enumerate((cp_w(0), [], [cp_wo], [cp_m[2]])):
            wait(copies)
            own_region(u, functools.partial(fill, u))

        def first_pair(i, _):
            for e in range(2):
                g = 2 * i + e
                wait(cp_w(g + 1))
                pl.when(g + 2 < NC)(lambda g=g: start(cp_w(g + 2)))
                own_region(e, functools.partial(
                    attn_block, g * _U, e, _NV_FIRST, 0, lambda u: None,
                    functools.partial(ffn_weights, g + 1), not (isinstance(g, int) and g == 0)))

        first_pair(0, None)
        lax.fori_loop(1, NPAIR, first_pair, None)

    vm = pltpu.VMEM
    pl.run_scoped(phase1, vm((D, D), dt), vm((8, DH, D), dt), vm((D, D), dt), vm((2, D, _CF), dt),
                  vm((2, D, _CF), dt), vm((2, D, _CF), dt), vm((32, 1, D), dt), vm((D, 6 * D), dt))

    def phase2(ahead_s, x1_s, h2_s, acc_s, out_s):
        ahead = ahead_s.bitcast(_BF)

        def heads(b, hi):
            return jnp.concatenate(
                [o_s[l, pl.ds(pl.multiple_of(b * HD, 8), hi // 2), :] for l in range(NL)], axis=1)

        def second_norm(b, attn, meanwhile):
            x1 = xt[b].astype(_F32) + _tile_lanes(modc[2 * D:3 * D, :]) * attn
            x1_s[...] = x1
            meanwhile()
            h2 = _layernorm(x1) * _tile_lanes(modc[4 * D:5 * D, :]) + _tile_lanes(modc[3 * D:4 * D, :])
            a11, a12, r1 = h2[0:256, :HT], h2[256:512, :HT], h2[512:D, :HT]
            a21, a22, r2 = h2[0:256, HT:], h2[256:512, HT:], h2[512:D, HT:]
            tiles = []
            for a, r in ((a11 + a22, r1), (a21 + a22, r2), (a11, r1), (a22, None), (a11 + a12, None),
                         (a21 - a11, r2 - r1), (a12 - a22, None)):
                tiles += [a] if r is None else [a[128:256], a[0:128], a[128:192], r, a[192:256], r]
            h2_s[...] = _pack(jnp.concatenate(tiles, axis=0).T)

        def ffn_chunks(j0, count, fresh, it=None, b=None):
            steps = -(-_H * _UF // NC)
            st = dict(done=0, share=0, round=0)
            mask = never()

            def next_ahead():
                n, r = divmod(st["done"], _NV_AHEAD)
                st["done"] += 1
                if r == 0:
                    h, l = jnp.minimum(it * steps + n // NL, _H - 1), n % NL
                    q = q_s.at[jnp.minimum((b + 1) * _H + _U + h, NB * _H - 1)]
                    st["p"] = vpu_weights(q, 0, _NV_AHEAD, l)
                    dst = ahead.at[jnp.where(h < _H - _U, h, h + _U * (b & 1))]
                    dst[:, 128 * l:128 * (l + 1)] = st["p"].reshape(8 * _NV_AHEAD, 128).astype(_BF)
                return st["p"][r]

            def tie(tiles, work):
                nr = tiles[0].shape[0] // 8
                rows = [[x[8 * i:8 * (i + 1)] for i in range(nr)] for x in tiles]
                used = [0] * nr

                def attach(i, v):
                    while used[i] == len(tiles):
                        i = (i + 1) % nr
                    rows[used[i]][i] = jnp.where(mask, pltpu.bitcast(v, _U32), rows[used[i]][i])
                    used[i] += 1

                if it is not None:
                    st["share"] += _SHARE[st["round"] % len(_SHARE)]
                    st["round"] += 1
                    n = steps * NL * _NV_AHEAD * st["share"] // (_UF * sum(_SHARE)) - st["done"]
                    for k in range(n):
                        attach((2 * k + 1) * nr // (2 * n), next_ahead())
                if work is not None:
                    n = work.shape[0] // 8
                    for k in range(n):
                        attach(k * nr // n, work[8 * k:8 * (k + 1)])
                return [jnp.concatenate(r, axis=0) for r in rows]

            def up_project(j, w, finish):
                out = []

                def wt(p, i, n):
                    return wgu[j, wbase[p] + 128 * i:wbase[p] + 128 * (i + n), 128 * w:128 * (w + 1)]

                def ht(p, i):
                    return h2_s[:, 128 * (hbase[p] + i):128 * (hbase[p] + i + 1)]

                shared = {p: _mm(_unpack(x), wt(p, 0, 1))
                          for p, x in zip(wide, tie([ht(p, 3) for p in wide], None))}

                def two(*pts):
                    hs = tie([ht(p, k + (t if p in wide else 0)) for p, t in pts for k in range(2)],
                             out[-1] if w and out else None)
                    ms = []
                    for n, (p, t) in enumerate(pts):
                        m = _mm(_unpack(jnp.concatenate(hs[2 * n:2 * n + 2], axis=1)),
                                wt(p, 2 * t + (p in wide), 2))
                        ms.append(m + shared[p] if p in wide else m)
                    return ms

                keep = []
                for t in range(2):
                    m2, m4 = two((1, t), (3, t))
                    out.append(finish(len(out), m2 + m4))
                    keep.append((m2, m4))
                for t in range(2):
                    m3, m5 = two((2, t), (4, t))
                    out.append(finish(len(out), m3 + m5))
                    keep[t] = (m3 - keep[t][0], keep[t][1] - m5)
                for t in range(2):
                    m1, m7 = two((0, t), (6, t))
                    out.append(finish(len(out), (keep[t][1] + m1) + m7))
                    keep[t] = keep[t][0] + m1
                for t, m6 in enumerate(two((5, 0), (5, 1))):
                    out.append(finish(len(out), keep[t] + m6))
                return out

            for dj in range(count):
                j = j0 + dj
                g = up_project(j, 0, lambda n, x: x)
                a = up_project(j, 1, lambda n, u: (g[n] * u) * (1.0 + jnp.tanh(g[n])))
                b12, b21, b11, b22 = [jnp.concatenate(a[2 * n:2 * n + 2], axis=1) for n in range(4)]
                for n, (p, x) in enumerate(((1, b11), (3, b21 - b11), (5, b11 + b12), (4, b22),
                                            (0, b11 + b22), (2, b12 - b22), (6, b21 + b22))):
                    w = pltpu.bitcast(wd[j, p * HD:(p + 1) * HD, :], _U32)
                    ws = [w[:, :128], w[:, 128:]]
                    if n < 2:
                        ws = tie(ws * 2, a[6 + n])
                        y = jnp.concatenate([
                            _mm_nt(_unpack(jnp.concatenate(ws[2 * t:2 * t + 2], axis=1)),
                                   x[128 * t:128 * (t + 1)]) for t in range(2)], axis=1)
                    else:
                        y = _mm_nt(_unpack(jnp.concatenate(tie(ws, None), axis=1)), x)
                    if dj > 0 or fresh is False:
                        y = y + acc_s[p]
                    elif fresh is not True:
                        y = y + jnp.where(fresh, 0.0, acc_s[p])
                    acc_s[p] = y

        def out_copy(b, i):
            rows = pl.ds(i * HD, HD)
            return pltpu.make_async_copy(
                out_s.at[b, rows], out_hbm.at[rows, pl.ds(pl.multiple_of(b * _TQ, _TQ), _TQ)],
                sem_out.at[2 * b + i])

        def ffn_result(b):
            m1, m2, m3, m4, m5, m6, m7 = [acc_s.at[p] for p in range(7)]
            for i in range(2):
                if i == 0:
                    y = [m1[...] + m4[...] - m5[...] + m7[...], m3[...] + m5[...]]
                else:
                    y = [m2[...] + m4[...], m1[...] - m2[...] + m3[...] + m6[...]]
                gate = _tile_lanes(modc[5 * D + i * HD:5 * D + (i + 1) * HD, :])
                out_s[b, i * HD:(i + 1) * HD] = (
                    x1_s[i * HD:(i + 1) * HD] + gate * jnp.concatenate(y, axis=1)).astype(dt)
                out_copy(b, i).start()

        def token_block(b, _):
            def later_queries(i, work):
                g = jnp.minimum(3 * b + i, 7)
                b2 = lax.shift_right_logical(g, 2) + 2
                w = wqt[pl.ds(pl.multiple_of((g & 3) * (4 * DH), 8), 4 * DH), :]
                put_q(b2 * _H + 4 * (g & 3), project(w, pltpu.bitcast(hb[b2], _U32), work))

            def consume(retry):
                del retry
                later_queries(0, [v for l in range(NL) for u in range(_U)
                                  for v in normalize((b + 1) * _H - _U + u, _U + u, l)])
                attn = project(pltpu.bitcast(wot[...], _U32), heads(b, D), [])
                second_norm(b, jnp.concatenate(attn, axis=0),
                            lambda: [later_queries(i, []) for i in (1, 2)])

            def block(i, e):
                h = (2 * i + e) * _U
                h2 = jnp.where(h > 0, h - _U, _H - _U * (b & 1))
                attn_block((b + 1) * _H + h, e, _NV_LATER, _NV_AHEAD, lambda u: ahead.at[h2 + u],
                           lambda u: [], True)

            def pair(i, _):
                block(i, 0)
                pl.when((b + 1) * NPAIR + i < NB * NPAIR - 1)(functools.partial(block, i, 1))

            guarded(b, consume)
            lax.fori_loop(0, NC // _UF, lambda i, _: ffn_chunks(i * _UF, _UF, i == 0, i, b), None)
            ffn_result(b)
            lax.fori_loop(0, NPAIR, pair, None)

        def last_consume(retry):
            early = _unpack(heads(NB - 1, 384))
            parts = []

            def piece():
                k, (a, b) = len(parts) // 4, _split(HD // 16, 4)[len(parts) % 4]
                parts.append(_mm(wot[16 * a:16 * b, 512 * k:512 * k + 384], early))

            for u in range(_U):
                for l in range(NL):
                    normalize(NB * _H - 2 * _U + u, u, l)
            for u in range(_U):
                num = attn_step(None, None, _U + u, 0, 0, ahead.at[_H - 2 * _U + u], [piece] * 2)
                n_s[_U + u] = jnp.where(retry, n_s[_U + u], num)
                for l in range(NL):
                    normalize(NB * _H - _U + u, _U + u, l)
            x = heads(NB - 1, D)
            p, q, r = x[192:224], x[224:256], x[256:HD]
            sh, top, bot = [_mm(wot[:, k:k + 128], _unpack(jnp.concatenate(xs, axis=0)))
                            for k, xs in ((1024, [r, q]), (384, [p, q]), (896, [p, r]))]
            attn = jnp.concatenate(parts, axis=0) + jnp.concatenate([top + sh, bot + sh], axis=0)
            second_norm(NB - 1, attn, lambda: None)
            ffn_chunks(0, 1, True)

        for u in range(_U):
            ahead.at[_H + u][...] = p_s[u, 0:8 * _NV_AHEAD, :].astype(_BF)
        lax.fori_loop(0, NB - 1, token_block, None)
        guarded(NB - 1, last_consume)
        lax.fori_loop(0, (NC - 1) // _UL, lambda i, _: ffn_chunks(1 + i * _UL, _UL, False), None)
        ffn_result(NB - 1)
        for b in range(NB):
            for i in range(2):
                out_copy(b, i).wait()

    pl.run_scoped(phase2, vm((_H + _U, 4 * _NV_AHEAD, _TQ), _U32), vm((D, _TQ), _F32),
                  vm((HT // 2, 22 * 128), _U32), vm((7, HD, HT), _F32), vm((NB, D, _TQ), dt))


@jax.jit
def pallas_adaLN_cond__grouped_kv_mqa__swiglu_ffn__prompt_kernel(
    A_x: jax.Array,
    A_wq: jax.Array,
    A_wk: jax.Array,
    A_wv: jax.Array,
    A_wo: jax.Array,
    B_x: jax.Array,
    B_w_gate: jax.Array,
    B_w_up: jax.Array,
    B_w_down: jax.Array,
    c: jax.Array,
    w_mod: jax.Array,
):
    del B_x
    _, S, D = A_x.shape
    F = B_w_gate.shape[1]
    assert (A_x.shape, F) == ((1, 2048, 576), 4608)
    NB = S // _TQ
    NC = F // _CF
    dt = A_x.dtype
    hbm = pl.BlockSpec(memory_space=pltpu.HBM)
    vm = pltpu.VMEM
    out_t = pl.pallas_call(
        _kernel,
        out_shape=jax.ShapeDtypeStruct((D, S), dt),
        in_specs=[hbm] * 10,
        out_specs=hbm,
        scratch_shapes=[
            vm((NB, D, _TQ), dt),
            vm((6 * D, 128), _F32),
            vm((D // 2, 2 * D), _F32),
            vm((2, D // 4, 2 * D), _U32),
            vm((NB, D // 2, _TQ), _U32),
            vm((NB * _H, 24, _TQ), _F32),
            vm((S, 24), _F32),
            vm((_NV_LATER + _NV_AHEAD, 20, 8, 128), _F32),
            vm((24, S), _F32),
            vm((2 * _U, S, _TQ), _F32),
            vm((2 * _U, 24, _TQ), _F32),
            vm((8, _TQ), _F32),
            vm((_TQ // 128, NB * D // 2 + 32, 128), _U32),
            vm((NC, 32 * 64, 256), _U32),
            vm((NC, 7 * D // 4, _CF // 2), _U32),
            pltpu.SMEM((8,), jnp.int32),
            pltpu.SemaphoreType.DMA((8,)),
            pltpu.SemaphoreType.DMA((NB,)),
            pltpu.SemaphoreType.DMA((NC,)),
            pltpu.SemaphoreType.DMA((2 * NB,)),
        ],
        compiler_params=pltpu.CompilerParams(vmem_limit_bytes=120 * 2 ** 20),
        name="adaln_mqa_swiglu",
    )(A_x.reshape(S, D).T, A_wq, A_wk.T, A_wv.T, A_wo, B_w_gate, B_w_up, B_w_down.T, c, w_mod)
    return out_t.T.reshape(1, S, D)
```

```python
import functools
import math

import jax
import jax.numpy as jnp
from jax import lax
import jax.experimental.pallas as pl
import jax.experimental.pallas.tpu as pltpu

_H = 32
_EPS = 1e-5
_TQ = 512
_CF = 512
_U = 4
_UF = 3
_UL = 2
_NV_FILL = (32, 32, 20, 20)
_NV_FIRST = 35
_NV_LATER = 38
_NV_AHEAD = 28
_SHARE = (22, 24, 24, 22, 20, 20, 16, 16, 20, 24, 16, 16, 16, 14, 12, 4, 9, 18, 15, 15, 15, 24, 24)
_SUM_LO, _SUM_HI = 2.0 ** -30, 2.0 ** 120

_BF = jnp.bfloat16
_F32 = jnp.float32
_U32 = jnp.uint32


def _mm(a, b):
    return lax.dot_general(a, b, (((1,), (0,)), ((), ())), preferred_element_type=_F32)


def _mm_nt(a, b):
    return lax.dot_general(a, b, (((1,), (1,)), ((), ())), preferred_element_type=_F32)


def _pack(x):
    return pltpu.bitcast(x.astype(_BF), _U32)


def _unpack(x):
    return pltpu.bitcast(x, _BF)


def _tile_lanes(col):
    return jnp.concatenate([col] * (_TQ // 128), axis=1)


def _tree_sum(xs):
    if len(xs) == 1:
        return xs[0]
    h = (len(xs) + 1) // 2
    return _tree_sum(xs[:h]) + _tree_sum(xs[h:])


def _split(n, parts):
    e = [(i * n + parts // 2) // parts for i in range(parts + 1)]
    return list(zip(e[:-1], e[1:]))


def _interleave(*lists):
    both = [((2 * i + 1) / len(t), x) for t in lists for i, x in enumerate(t)]
    return [x for _, x in sorted(both, key=lambda e: e[0])]


def _layernorm(x):
    d = x.shape[0]
    xc = x - jnp.sum(x, axis=0, keepdims=True) * (1.0 / d)
    var = jnp.sum(xc * xc, axis=0, keepdims=True) * (1.0 / d)
    return xc * lax.rsqrt(var + _EPS)


def _kernel(xt_hbm, wq_hbm, wkt_hbm, wvt_hbm, wo_hbm, wg_hbm, wu_hbm, wdt_hbm, c_hbm, wmod_hbm,
            out_hbm,
            xt, modc, wqt, wot, h_s, q_s, k_s, kb_s, vt_s, p_s, n_s, bad_s, o_s, wgu, wd,
            zero_s, sem_in, sem_x, sem_w, sem_out):
    D, S = xt_hbm.shape
    F = wg_hbm.shape[1]
    dt = xt_hbm.dtype
    DH = D // _H
    DP = q_s.shape[1]
    HD = D // 2
    HT = _TQ // 2
    NB = S // _TQ
    NC = F // _CF
    NL = _TQ // 128
    NPAIR = _H // (2 * _U)
    wide = (1, 2, 0, 5)
    wbase = [0, 640, 1280, 1920, 2432, 2944, 3584]
    hbase = [0, 4, 8, 12, 14, 16, 20]

    def never():
        return jnp.full((8, 128), zero_s[0], jnp.int32) > 0

    def own_region(i, fn):
        pl.when(zero_s[1 + i] == 0)(fn)

    def put_weights(ref, w):
        w = w.astype(_F32)
        w = jnp.concatenate([w, w[512:D]], axis=0).T
        a, b = w[:HD], w[HD:]
        low = lax.broadcasted_iota(jnp.int32, (HD, 128), 1) < 64
        w = jnp.concatenate(
            [a[:, 0:384], jnp.where(low, a[:, 384:512], a[:, 384:512] - b[:, 384:512]),
             b[:, 0:384], jnp.where(low, b[:, 384:512], b[:, 512:640] - a[:, 512:640]),
             jnp.where(low, a[:, 512:640], b[:, 384:512])], axis=1)
        ref[:, 0:2 * D] = _pack(w) if ref.dtype == _U32 else w

    def project(w, x, work):
        mask = never()
        nr = w.shape[0] // 8
        view = _unpack if w.dtype == _U32 else lambda v: v

        def streamed(k, vs):
            rows = [w[8 * i:8 * (i + 1), k:k + 128] for i in range(nr)]
            for i, (a, b) in enumerate(_split(len(vs), nr)):
                if b > a:
                    rows[i] = jnp.where(mask, functools.reduce(jnp.maximum, vs[a:b]), rows[i])
            return view(jnp.concatenate(
                [jnp.concatenate(rows, axis=0), w[:, k + 128:k + 512]], axis=1))

        shared = _mm(view(w[:, 1024:1152]), _unpack(jnp.concatenate([x[256:HD], x[224:256]], axis=0)))
        cols = []
        for l, (lo, hi) in enumerate(_split(len(work), NL)):
            xl, sh = [v[:, 128 * l:128 * (l + 1)] for v in (x, shared)]
            mid = (lo + hi) // 2
            cols.append((
                _mm(streamed(0, work[lo:mid]), _unpack(xl[0:256])) + sh,
                _mm(streamed(512, work[mid:hi]),
                    _unpack(jnp.concatenate([xl[0:224], xl[256:HD]], axis=0))) + sh))
        return [jnp.concatenate(c, axis=1) for c in zip(*cols)]

    def put_q(t, halves):
        for n, q in enumerate(halves):
            heads = q.shape[0] // DH
            q = jnp.concatenate([q, jnp.zeros((8, _TQ), _F32)], axis=0)
            for i in range(heads):
                q_s[t + n * (_H // 2) + i] = q[DH * i:DH * i + DP]

    def put_o(t, l, num):
        o = num * (1.0 / num[DH:DH + 1, :])
        o = _pack(jnp.concatenate([o, jnp.zeros((8, 128), _F32)], axis=0))
        o_s[l, pl.ds(t * (DH // 2), 16), :] = o
        return o

    def vpu_weights(q, lo, hi, l):
        return jnp.exp2(_tree_sum([
            kb_s[lo:hi, d] * jnp.broadcast_to(q[d:d + 1, 128 * l:128 * (l + 1)], (8, 128))
            for d in range(DH)]))

    def attn_step(t, dst, src, n_vpu, n_ahead, ahead, work):
        lo = n_vpu + n_ahead
        n_mxu = S // 8 - lo
        n_rows = n_mxu + (0 if src is None else S // 128 * DP // 8)
        due = {}
        row = [0]
        mask = never()

        def spread(fns):
            for n, fn in enumerate(fns):
                due.setdefault((2 * n + 1) * n_rows // (2 * len(fns)), []).append(fn)

        def tied(x):
            rows = []
            for i in range(0, x.shape[0], 8):
                vs = [v for fn in due.get(row[0], []) for v in fn()]
                row[0] += 1
                rows.append(x[i:i + 8])
                if vs:
                    v = functools.reduce(jnp.maximum, vs)
                    rows[-1] = jnp.where(mask[:, :x.shape[1]], v[:, :x.shape[1]], rows[-1])
            return jnp.concatenate(rows, axis=0)

        def weights(a, b):
            cut = a if ahead is None else min(max(8 * _NV_AHEAD, a), b)
            if cut == a:
                return p_s[src, a:b, :]
            if cut == b:
                return ahead[a:b, :]
            return jnp.concatenate([ahead[a:cut, :].astype(_F32), p_s[src, cut:b, :]], axis=0)

        if t is not None:
            q = q_s.at[t]
            vpu = []
            for l in range(NL):
                p = vpu_weights(q, n_ahead, lo, l)
                p_s[dst, 8 * n_ahead:8 * lo, 128 * l:128 * (l + 1)] = p.reshape(8 * n_vpu, 128)
                vpu += [lambda v=p[r]: [v] for r in range(n_vpu)]
            spread(vpu)
            spread([lambda fn=fn: fn()[::-4] for fn in work])
        num = None
        for c, (a, b) in enumerate(_split(n_mxu, S // 128)):
            if t is not None:
                keys = slice(8 * (lo + a), 8 * (lo + b))
                p_s[dst, keys, :] = jnp.exp2(_mm(tied(k_s[keys, :]), q[...]))
            elif c % 8 == 0:
                work[c // 8]()
            if src is not None:
                r = _mm(tied(vt_s[:, 128 * c:128 * (c + 1)]), weights(128 * c, 128 * (c + 1)))
                num = r if c == 0 else num + r
        return num

    def normalize(t, slot, l):
        lanes = slice(128 * l, 128 * (l + 1))
        num = n_s[slot, :, lanes]
        safe = (num[DH:DH + 1, :] >= _SUM_LO) & functools.reduce(
            jnp.logical_and, [jnp.abs(num[i:i + 8]) <= _SUM_HI for i in range(0, DP, 8)])
        bad = jnp.where(safe, bad_s[:, lanes], 1.0)
        bad_s[:, lanes] = bad
        o = pltpu.bitcast(put_o(t, l, num), _F32)
        return [bad, o[0:8], o[8:16]]

    def attn_block(t, e, n_vpu, n_ahead, ahead_of, work_of, pending):
        for u in range(_U):
            this, other = e * _U + u, (1 - e) * _U + u
            norm = [functools.partial(normalize, t - _U + u, other, l)
                    for l in range(NL if pending else 0)]
            n_s[this] = attn_step(t + _U + u, other, this, n_vpu, n_ahead, ahead_of(u),
                                  _interleave(work_of(u), norm))

    def guarded(b, consume):
        def exact(n, _):
            h = lax.shift_right_logical(n, 2)
            l = n & (NL - 1)
            lanes = pl.ds(pl.multiple_of(128 * l, 128), 128)
            s = _mm(k_s[...], q_s[b * _H + h, :, lanes])
            num = _mm(vt_s[...], jnp.exp2(s - jnp.max(s, axis=0, keepdims=True)))
            n_s[h & (2 * _U - 1), :, lanes] = num
            put_o(b * _H + h, l, num)

        def attempt(state):
            retry = state > 0
            pl.when(retry)(lambda: lax.fori_loop(0, _H * NL, exact, None))
            consume(retry)
            unsafe = jnp.max(bad_s[...]) > 0.0
            bad_s[...] = jnp.zeros(bad_s.shape, _F32)
            return jnp.where(unsafe, state + 1, 2)

        lax.while_loop(lambda state: state < 2, attempt, jnp.int32(0))

    def phase1(wq, wkv_s, wo, wg, wu, wdt, cv_s, wmod):
        wkt, wvt, cv = wkv_s.at[0], wkv_s.at[1], cv_s.at[0]
        cp_c, cp_wk, cp_wv, cp_wq, cp_wo = [
            pltpu.make_async_copy(src, dst, sem_in.at[i]) for i, (src, dst) in enumerate(
                ((c_hbm, cv), (wkt_hbm, wkt), (wvt_hbm, wvt), (wq_hbm, wq), (wo_hbm, wo)))]
        mcut = (0, 512, 2 * D, 6 * D)
        cp_m = [pltpu.make_async_copy(wmod_hbm.at[:, pl.ds(a, b - a)], wmod.at[:, pl.ds(a, b - a)],
                                      sem_in.at[5 + i])
                for i, (a, b) in enumerate(zip(mcut, mcut[1:]))]
        cp_x = [pltpu.make_async_copy(xt_hbm.at[:, pl.ds(b * _TQ, _TQ)], xt.at[b], sem_x.at[b])
                for b in range(NB)]

        def cp_w(j):
            cols = pl.ds(pl.multiple_of(j * _CF, _CF), _CF)
            return [pltpu.make_async_copy(src.at[:, cols], dst.at[j & 1], sem_w.at[j])
                    for src, dst in ((wg_hbm, wg), (wu_hbm, wu), (wdt_hbm, wdt))]

        def start(copies):
            for cp in copies:
                cp.start()

        def wait(copies):
            for cp in copies:
                cp.wait()

        def mod_cols(sc, lo, hi):
            row = _mm(sc, wmod[:, lo:hi])[0:1, :]
            col = lax.broadcasted_iota(jnp.int32, row.shape, 1) + lo
            one = ((col >= D) & (col < 2 * D)) | ((col >= 4 * D) & (col < 5 * D))
            row = jnp.where(one, row + 1.0, row)
            row = row * jnp.where(col >= 5 * D, 2.0, jnp.where(col >= 3 * D, 0.5, 1.0))
            modc[lo:hi, :] = jnp.broadcast_to(row, (128, hi - lo)).T
            return []

        def ffn_weights(j, i):
            def rows(ref, base):
                x = ref[j & 1, base + 16 * i:base + 16 * (i + 1), :].astype(_F32)
                return [x[:, 128 * t:128 * (t + 1)] for t in range(4)]

            def put(ref, tiles):
                val = _pack(jnp.concatenate([v for _, _, v in tiles], axis=1))
                val = [val[:, 128 * n:128 * (n + 1)] for n in range(len(tiles))]
                for (row, lane, _), v in zip(tiles, val):
                    ref[j, row // 2:row // 2 + 8, 128 * lane:128 * (lane + 1)] = v
                return [pltpu.bitcast(v, _F32) for v in val]

            def main_part(w, ref, r0):
                top, bot = rows(ref, r0), rows(ref, 256 + r0)
                sums = [[b11 + b22, b11, b12 - b22, b21 - b11, b22, b11 + b12, b21 + b22]
                        for b11, b12, b21, b22
                        in ((top[t], top[t + 2], bot[t], bot[t + 2]) for t in range(2))]
                out = []
                for p, (va, vb) in enumerate(zip(*sums)):
                    if p not in wide:
                        out += [(wbase[p] + r0, va), (wbase[p] + 256 + r0, vb)]
                    elif r0 < 128:
                        out += [(wbase[p] + 256 + r0, va), (wbase[p] + 384 + r0, vb)]
                    elif r0 == 128:
                        out += [(wbase[p] + 128, va), (wbase[p] + 512, vb)]
                    else:
                        out += [(wbase[p], vb), (wbase[p] + 192, va - vb)]
                return put(wgu, [(r + 16 * i, w, v) for r, v in out])

            def rest_part(w, ref):
                r = rows(ref, 512)
                out = []
                for p, va, vb in ((0, r[0], r[1]), (1, r[0], r[1]), (2, r[2], r[3]),
                                  (5, r[0] + r[2], r[1] + r[3])):
                    out += [(wbase[p] + 64, va), (wbase[p] + 576, vb - va)]
                return put(wgu, [(r + 16 * i, w, v) for r, v in out])

            def down_part(g):
                top = wdt[j & 1, 16 * g:16 * (g + 1), :].astype(_F32)
                bot = wdt[j & 1, HD + 16 * g:HD + 16 * (g + 1), :].astype(_F32)
                a11, a12, a21, a22 = top[:, :256], top[:, 256:], bot[:, :256], bot[:, 256:]
                sums = (a11 + a22, a21 + a22, a11, a22, a11 + a12, a21 - a11, a12 - a22)
                return put(wd, [(p * HD + 16 * g, t, v[:, 128 * t:128 * (t + 1)])
                                for p, v in enumerate(sums) for t in range(2)])

            fns = []
            for w, ref in enumerate((wg, wu)):
                fns += [functools.partial(main_part, w, ref, r0) for r0 in (0, 64, 128, 192)]
                fns.append(functools.partial(rest_part, w, ref))
            return fns + [functools.partial(down_part, g) for g in range(*_split(HD // 16, 4)[i])]

        def modulate(b):
            h = _pack(_layernorm(xt[b].astype(_F32)) * _tile_lanes(modc[D:2 * D, :])
                      + _tile_lanes(modc[0:D, :]))
            h_s[b] = h
            return [pltpu.bitcast(h[i:i + 8, 128 * l:128 * (l + 1)], _F32)
                    for l in range(NL) for i in range(0, HD, 8)]

        def keys_values(b, centre=None):
            zpad = jnp.zeros((DP - DH, D), _F32)
            wkv = jnp.concatenate([wkt[...].astype(_F32), zpad, wvt[...].astype(_F32), zpad], axis=0)
            kv = _mm(wkv, _unpack(h_s[b]))
            kt = kv[0:DP] * (DH ** -0.5 * math.log2(math.e))
            k = jnp.concatenate([kt, jnp.zeros((128 - DP, _TQ), _F32)], axis=0).T[:, 0:DP]
            if centre is None:
                centre = jnp.sum(k, axis=0, keepdims=True) * (1.0 / _TQ)
            k_s[b * _TQ:(b + 1) * _TQ, :] = k - centre
            rows = lax.broadcasted_iota(jnp.int32, (DP, _TQ), 0)
            vt_s[:, b * _TQ:(b + 1) * _TQ] = jnp.where(rows < DH, kv[DP:], 1.0)
            return centre

        def spread_keys(lo, hi):
            k = k_s[8 * lo:8 * hi, :]
            cols = [jnp.broadcast_to(k[:, d:d + 1], (8 * (hi - lo), 128)).reshape(hi - lo, 8, 128)
                    for d in range(DH)]
            for d in range(DH):
                kb_s[lo:hi, d] = cols[d]
            return [lambda c=c: [c[hi - lo - 1]] for c in cols]

        def queries(b, work):
            put_q(b * _H, project(wqt[...], h_s[b], work))

        start([cp_c, cp_m[0], cp_m[1], cp_wk, cp_wv])
        for i in range(zero_s.shape[0]):
            zero_s[i] = 0
        bad_s[...] = jnp.zeros(bad_s.shape, _F32)
        cp_c.wait()
        cf = cv[...].astype(_F32)
        sc = jnp.broadcast_to(cf * jax.nn.sigmoid(cf), (8, D))
        cp_m[0].wait()
        cp_wq.start()
        mod_cols(sc, mcut[0], mcut[1])
        cp_m[1].wait()
        cp_x[0].start()
        mod_cols(sc, mcut[1], mcut[2])
        cp_wq.wait()
        cp_x[1].start()
        put_weights(wqt, wq[...])

        start(cp_x[2:])
        wait([cp_wk, cp_wv, cp_x[0]])
        modulate(0)
        centre = keys_values(0)
        n_ready = max(_NV_FILL)
        spread_keys(0, n_ready)
        queries(0, [])

        start(cp_w(0))
        wait(cp_x[1:])
        start([cp_wo, cp_m[2]])
        modulate(1)
        keys_values(1, centre)
        queries(1, [v for b in range(2, NB) for v in modulate(b)])
        for b in range(2, NB):
            keys_values(b, centre)

        def fill(u):
            if u < 2:
                more = spread_keys(*(n_ready + x for x in _split(kb_s.shape[0] - n_ready, 2)[u]))
            elif u == 2:
                put_weights(wot, wo[...])
                more = [lambda i=i, k=k: [pltpu.bitcast(wot[i:i + 8, k:k + 128], _F32)]
                        for k in (0, 512, 128, 640, 256, 768, 384, 896, 1024) for i in (56, 120)]
            else:
                more = [functools.partial(mod_cols, sc, k, k + 128) for k in range(2 * D, 6 * D, 128)]
            attn_step(u, u, None, _NV_FILL[u], 0, None, _interleave(ffn_weights(0, u), more))

        start(cp_w(1))
        for u, copies in enumerate((cp_w(0), [], [cp_wo], [cp_m[2]])):
            wait(copies)
            own_region(u, functools.partial(fill, u))

        def first_pair(i, _):
            for e in range(2):
                g = 2 * i + e
                wait(cp_w(g + 1))
                pl.when(g + 2 < NC)(lambda g=g: start(cp_w(g + 2)))
                own_region(e, functools.partial(
                    attn_block, g * _U, e, _NV_FIRST, 0, lambda u: None,
                    functools.partial(ffn_weights, g + 1), not (isinstance(g, int) and g == 0)))

        first_pair(0, None)
        lax.fori_loop(1, NPAIR, first_pair, None)

    vm = pltpu.VMEM
    pl.run_scoped(phase1, vm((D, D), dt), vm((8, DH, D), dt), vm((D, D), dt), vm((2, D, _CF), dt),
                  vm((2, D, _CF), dt), vm((2, D, _CF), dt), vm((32, 1, D), dt), vm((D, 6 * D), dt))

    def phase2(ahead, x1_s, h2_s, acc_s, out_s):
        def heads(b, hi):
            return jnp.concatenate(
                [o_s[l, pl.ds(pl.multiple_of(b * HD, 8), hi // 2), :] for l in range(NL)], axis=1)

        def second_norm(b, attn, meanwhile):
            x1 = xt[b].astype(_F32) + _tile_lanes(modc[2 * D:3 * D, :]) * attn
            x1_s[...] = x1
            meanwhile()
            h2 = _layernorm(x1) * _tile_lanes(modc[4 * D:5 * D, :]) + _tile_lanes(modc[3 * D:4 * D, :])
            a11, a12, r1 = h2[0:256, :HT], h2[256:512, :HT], h2[512:D, :HT]
            a21, a22, r2 = h2[0:256, HT:], h2[256:512, HT:], h2[512:D, HT:]
            tiles = []
            for a, r in ((a11 + a22, r1), (a21 + a22, r2), (a11, r1), (a22, None), (a11 + a12, None),
                         (a21 - a11, r2 - r1), (a12 - a22, None)):
                tiles += [a] if r is None else [a[128:256], a[0:128], a[128:192], r, a[192:256], r]
            h2_s[...] = _pack(jnp.concatenate(tiles, axis=0).T)

        def ffn_chunks(j0, count, fresh, it=None, b=None):
            steps = -(-_H * _UF // NC)
            st = dict(done=0, share=0, round=0)
            mask = never()

            def next_ahead():
                n, r = divmod(st["done"], _NV_AHEAD)
                st["done"] += 1
                if r == 0:
                    h, l = jnp.minimum(it * steps + n // NL, _H - 1), n % NL
                    q = q_s.at[jnp.minimum((b + 1) * _H + _U + h, NB * _H - 1)]
                    st["p"] = vpu_weights(q, 0, _NV_AHEAD, l)
                    dst = ahead.at[jnp.where(h < _H - _U, h, h + _U * (b & 1))]
                    dst[:, 128 * l:128 * (l + 1)] = st["p"].reshape(8 * _NV_AHEAD, 128).astype(_BF)
                return st["p"][r]

            def tie(tiles, work):
                nr = tiles[0].shape[0] // 8
                rows = [[x[8 * i:8 * (i + 1)] for i in range(nr)] for x in tiles]
                used = [0] * nr

                def attach(i, v):
                    while used[i] == len(tiles):
                        i = (i + 1) % nr
                    rows[used[i]][i] = jnp.where(mask, pltpu.bitcast(v, _U32), rows[used[i]][i])
                    used[i] += 1

                if it is not None:
                    st["share"] += _SHARE[st["round"] % len(_SHARE)]
                    st["round"] += 1
                    n = steps * NL * _NV_AHEAD * st["share"] // (_UF * sum(_SHARE)) - st["done"]
                    for k in range(n):
                        attach((2 * k + 1) * nr // (2 * n), next_ahead())
                if work is not None:
                    n = work.shape[0] // 8
                    for k in range(n):
                        attach(k * nr // n, work[8 * k:8 * (k + 1)])
                return [jnp.concatenate(r, axis=0) for r in rows]

            def up_project(j, w, finish):
                out = []

                def wt(p, i, n):
                    r = wbase[p] // 2 + 64 * i
                    return _unpack(wgu[j, r:r + 64 * n, 128 * w:128 * (w + 1)])

                def ht(p, i):
                    return h2_s[:, 128 * (hbase[p] + i):128 * (hbase[p] + i + 1)]

                shared = {p: _mm(_unpack(x), wt(p, 0, 1))
                          for p, x in zip(wide, tie([ht(p, 3) for p in wide], None))}

                def two(*pts):
                    hs = tie([ht(p, k + (t if p in wide else 0)) for p, t in pts for k in range(2)],
                             out[-1] if w and out else None)
                    ms = []
                    for n, (p, t) in enumerate(pts):
                        m = _mm(_unpack(jnp.concatenate(hs[2 * n:2 * n + 2], axis=1)),
                                wt(p, 2 * t + (p in wide), 2))
                        ms.append(m + shared[p] if p in wide else m)
                    return ms

                keep = []
                for t in range(2):
                    m2, m4 = two((1, t), (3, t))
                    out.append(finish(len(out), m2 + m4))
                    keep.append((m2, m4))
                for t in range(2):
                    m3, m5 = two((2, t), (4, t))
                    out.append(finish(len(out), m3 + m5))
                    keep[t] = (m3 - keep[t][0], keep[t][1] - m5)
                for t in range(2):
                    m1, m7 = two((0, t), (6, t))
                    out.append(finish(len(out), (keep[t][1] + m1) + m7))
                    keep[t] = keep[t][0] + m1
                for t, m6 in enumerate(two((5, 0), (5, 1))):
                    out.append(finish(len(out), keep[t] + m6))
                return out

            for dj in range(count):
                j = j0 + dj
                g = up_project(j, 0, lambda n, x: x)
                a = up_project(j, 1, lambda n, u: (g[n] * u) * (1.0 + jnp.tanh(g[n])))
                b12, b21, b11, b22 = [jnp.concatenate(a[2 * n:2 * n + 2], axis=1) for n in range(4)]
                for n, (p, x) in enumerate(((1, b11), (3, b21 - b11), (5, b11 + b12), (4, b22),
                                            (0, b11 + b22), (2, b12 - b22), (6, b21 + b22))):
                    w = wd[j, p * HD // 2:(p + 1) * HD // 2, :]
                    ws = [w[:, :128], w[:, 128:]]
                    if n < 2:
                        ws = tie(ws * 2, a[6 + n])
                        y = jnp.concatenate([
                            _mm_nt(_unpack(jnp.concatenate(ws[2 * t:2 * t + 2], axis=1)),
                                   x[128 * t:128 * (t + 1)]) for t in range(2)], axis=1)
                    else:
                        y = _mm_nt(_unpack(jnp.concatenate(tie(ws, None), axis=1)), x)
                    if dj > 0 or fresh is False:
                        y = y + acc_s[p]
                    elif fresh is not True:
                        y = y + jnp.where(fresh, 0.0, acc_s[p])
                    acc_s[p] = y

        def out_copy(b, i):
            rows = pl.ds(i * HD, HD)
            return pltpu.make_async_copy(
                out_s.at[b, rows], out_hbm.at[rows, pl.ds(pl.multiple_of(b * _TQ, _TQ), _TQ)],
                sem_out.at[2 * b + i])

        def ffn_result(b):
            m1, m2, m3, m4, m5, m6, m7 = [acc_s.at[p] for p in range(7)]
            for i in range(2):
                if i == 0:
                    y = [m1[...] + m4[...] - m5[...] + m7[...], m3[...] + m5[...]]
                else:
                    y = [m2[...] + m4[...], m1[...] - m2[...] + m3[...] + m6[...]]
                gate = _tile_lanes(modc[5 * D + i * HD:5 * D + (i + 1) * HD, :])
                out_s[b, i * HD:(i + 1) * HD] = (
                    x1_s[i * HD:(i + 1) * HD] + gate * jnp.concatenate(y, axis=1)).astype(dt)
                out_copy(b, i).start()

        def token_block(b, _):
            def later_queries(i, work):
                g = jnp.minimum(3 * b + i, 7)
                b2 = lax.shift_right_logical(g, 2) + 2
                w = wqt[pl.ds(pl.multiple_of((g & 3) * (4 * DH), 8), 4 * DH), :]
                put_q(b2 * _H + 4 * (g & 3), project(w, h_s[b2], work))

            def consume(retry):
                del retry
                later_queries(0, [v for l in range(NL) for u in range(_U)
                                  for v in normalize((b + 1) * _H - _U + u, _U + u, l)])
                attn = project(wot[:, 0:2 * D], heads(b, D), [])
                second_norm(b, jnp.concatenate(attn, axis=0),
                            lambda: [later_queries(i, []) for i in (1, 2)])

            def block(i, e):
                h = (2 * i + e) * _U
                h2 = jnp.where(h > 0, h - _U, _H - _U * (b & 1))
                attn_block((b + 1) * _H + h, e, _NV_LATER, _NV_AHEAD, lambda u: ahead.at[h2 + u],
                           lambda u: [], True)

            def pair(i, _):
                block(i, 0)
                pl.when((b + 1) * NPAIR + i < NB * NPAIR - 1)(functools.partial(block, i, 1))

            guarded(b, consume)
            lax.fori_loop(0, NC // _UF, lambda i, _: ffn_chunks(i * _UF, _UF, i == 0, i, b), None)
            ffn_result(b)
            lax.fori_loop(0, NPAIR, pair, None)

        def last_consume(retry):
            early = _unpack(heads(NB - 1, 384))
            parts = []

            def piece():
                k, (a, b) = len(parts) // 4, _split(HD // 16, 4)[len(parts) % 4]
                parts.append(_mm(_unpack(wot[8 * a:8 * b, 512 * k:512 * k + 384]), early))

            for u in range(_U):
                for l in range(NL):
                    normalize(NB * _H - 2 * _U + u, u, l)
            for u in range(_U):
                num = attn_step(None, None, _U + u, 0, 0, ahead.at[_H - 2 * _U + u], [piece] * 2)
                n_s[_U + u] = jnp.where(retry, n_s[_U + u], num)
                for l in range(NL):
                    normalize(NB * _H - _U + u, _U + u, l)
            x = heads(NB - 1, D)
            p, q, r = x[192:224], x[224:256], x[256:HD]
            sh, top, bot = [_mm(_unpack(wot[:, k:k + 128]), _unpack(jnp.concatenate(xs, axis=0)))
                            for k, xs in ((1024, [r, q]), (384, [p, q]), (896, [p, r]))]
            attn = jnp.concatenate(parts, axis=0) + jnp.concatenate([top + sh, bot + sh], axis=0)
            second_norm(NB - 1, attn, lambda: None)
            ffn_chunks(0, 1, True)

        for u in range(_U):
            ahead.at[_H + u][...] = p_s[u, 0:8 * _NV_AHEAD, :].astype(_BF)
        lax.fori_loop(0, NB - 1, token_block, None)
        guarded(NB - 1, last_consume)
        lax.fori_loop(0, (NC - 1) // _UL, lambda i, _: ffn_chunks(1 + i * _UL, _UL, False), None)
        ffn_result(NB - 1)
        for b in range(NB):
            for i in range(2):
                out_copy(b, i).wait()

    pl.run_scoped(phase2, vm((_H + _U, 8 * _NV_AHEAD, _TQ), _BF), vm((D, _TQ), _F32),
                  vm((HT // 2, 22 * 128), _U32), vm((7, HD, HT), _F32), vm((NB, D, _TQ), dt))


@jax.jit
def pallas_adaLN_cond__grouped_kv_mqa__swiglu_ffn__prompt_kernel(
    A_x: jax.Array,
    A_wq: jax.Array,
    A_wk: jax.Array,
    A_wv: jax.Array,
    A_wo: jax.Array,
    B_x: jax.Array,
    B_w_gate: jax.Array,
    B_w_up: jax.Array,
    B_w_down: jax.Array,
    c: jax.Array,
    w_mod: jax.Array,
):
    del B_x
    _, S, D = A_x.shape
    F = B_w_gate.shape[1]
    assert (A_x.shape, F) == ((1, 2048, 576), 4608)
    NB = S // _TQ
    NC = F // _CF
    dt = A_x.dtype
    hbm = pl.BlockSpec(memory_space=pltpu.HBM)
    vm = pltpu.VMEM
    out_t = pl.pallas_call(
        _kernel,
        out_shape=jax.ShapeDtypeStruct((D, S), dt),
        in_specs=[hbm] * 10,
        out_specs=hbm,
        scratch_shapes=[
            vm((NB, D, _TQ), dt),
            vm((6 * D, 128), _F32),
            vm((D // 2, 2 * D), _F32),
            vm((D // 4, 2 * D + 128), _U32),
            vm((NB, D // 2, _TQ), _U32),
            vm((NB * _H, 24, _TQ), _F32),
            vm((S, 24), _F32),
            vm((_NV_LATER + _NV_AHEAD, 20, 8, 128), _F32),
            vm((24, S), _F32),
            vm((2 * _U, S, _TQ), _F32),
            vm((2 * _U, 24, _TQ), _F32),
            vm((8, _TQ), _F32),
            vm((_TQ // 128, NB * D // 2 + 32, 128), _U32),
            vm((NC, 32 * 64, 256), _U32),
            vm((NC, 7 * D // 4, _CF // 2), _U32),
            pltpu.SMEM((8,), jnp.int32),
            pltpu.SemaphoreType.DMA((8,)),
            pltpu.SemaphoreType.DMA((NB,)),
            pltpu.SemaphoreType.DMA((NC,)),
            pltpu.SemaphoreType.DMA((2 * NB,)),
        ],
        compiler_params=pltpu.CompilerParams(vmem_limit_bytes=120 * 2 ** 20),
        name="adaln_mqa_swiglu",
    )(A_x.reshape(S, D).T, A_wq, A_wk.T, A_wv.T, A_wo, B_w_gate, B_w_up, B_w_down.T, c, w_mod)
    return out_t.T.reshape(1, S, D)
```
